```python
import os as _os
_os.environ.setdefault("JAX_PLATFORMS", "cpu")
import jax
import jax.numpy as jnp

def _softmax(x, axis=-1):
    return jax.nn.softmax(x, axis=axis)
def _gelu(x):
    return jax.nn.gelu(x, approximate=True)
def _silu(x):
    return jax.nn.silu(x)
def _sigmoid(x):
    return jax.nn.sigmoid(x)
def _layernorm(x, axis=-1, eps=1e-5):
    m = jnp.mean(x, axis=axis, keepdims=True)
    v = jnp.var(x, axis=axis, keepdims=True)
    return (x - m) / jnp.sqrt(v + eps)
def _scatter_add(tgt, idx, src, axis=0):
    return tgt.at[idx].add(src)
def _segment_sum(src, seg, n):
    return jax.ops.segment_sum(src, seg, n)
class _Rng:
    def __init__(self, key):
        self._k = key
    def _next(self):
        self._k, sub = jax.random.split(self._k)
        return sub
    def normal(self, shape):
        return jax.random.normal(self._next(), shape, dtype=jnp.bfloat16)
    def randint(self, lo, hi, shape):
        return jax.random.randint(self._next(), shape, lo, hi, dtype=jnp.int32)
    def uniform(self, shape, lo=0.0, hi=1.0):
        return jax.random.uniform(self._next(), shape, jnp.bfloat16, lo, hi)
    def permutation(self, n):
        return jax.random.permutation(self._next(), n)


kernel_name = 'gated_mix__mha_block__ssm_conv_h3__prompt'

def setup_inputs():
    _rng = _Rng(jax.random.key(int.from_bytes(__import__("os").urandom(4), "little")))
    _w = (lambda a: (lambda t: t.astype(jnp.bfloat16) if jnp.issubdtype(t.dtype, jnp.floating) else t)(jnp.asarray(a)))
    def _A_setup():
        B, S, D, H = 1, 2048, 640, 32
        return {
            "x": _w((lambda *s: _rng.normal(s) * 0.05)(B, S, D)),
            "wqkv": _w((lambda *s: _rng.normal(s) * 0.4)(D, 3 * D)),
            "wo": _w((lambda *s: _rng.normal(s) * 0.05)(D, D)),
        }
    _A_in = _A_setup()

    def _B_setup():
        B, S, D = 1, 2048, 640
        ks = 4
        return {
            "q": _w((lambda *s: _rng.normal(s) * 0.05)(B, S, D)),
            "k": _w((lambda *s: _rng.normal(s) * 0.4)(B, S, D)),
            "v": _w((lambda *s: _rng.normal(s) * 0.4)(B, S, D)),
            "shift_k": _w((lambda *s: _rng.normal(s) * 0.4)(D, ks) * 0.5),
            "ssm_k": _w((lambda *s: _rng.normal(s) * 0.4)(D, S) * (1.0 / S ** 0.5)),
            "ssm_D": _w((lambda *s: _rng.normal(s) * 0.4)(D)),
        }
    _B_in = _B_setup()

    return {
        "A_x": _A_in["x"],
        "A_wqkv": _A_in["wqkv"],
        "A_wo": _A_in["wo"],
        "B_q": _B_in["q"],
        "B_k": _B_in["k"],
        "B_v": _B_in["v"],
        "B_shift_k": _B_in["shift_k"],
        "B_ssm_k": _B_in["ssm_k"],
        "B_ssm_D": _B_in["ssm_D"],
        "gate_w": _w((lambda *s: _rng.normal(s) * 0.05)(640) * 16.0),
    }

def reference(A_x, A_wqkv, A_wo, B_q, B_k, B_v, B_shift_k, B_ssm_k, B_ssm_D, gate_w):
    def _A_ref(x, wqkv, wo):
        B, S, D = x.shape
        H = 32
        Dh = D // H
        qkv = (lambda x, *d: x.transpose(*d))((x @ wqkv).reshape(B, S, 3, H, Dh), 2, 0, 3, 1, 4)
        q, k, v = qkv[0], qkv[1], qkv[2]
        scores = jnp.einsum("bhqd,bhkd->bhqk", q, k) * (Dh ** -0.5)
        p = _softmax(scores, axis=-1)
        o = jnp.einsum("bhqk,bhkd->bhqd", p, v)
        return (lambda x, *d: x.transpose(*d))(o, 0, 2, 1, 3).reshape(B, S, D) @ wo

    def _B_ref(q, k, v, shift_k, ssm_k, ssm_D):
        B, S, D = q.shape
        ks = shift_k.shape[-1]
        k_pad = jnp.pad(k, ((0, 0), (ks - 1, 0), (0, 0)))
        k_shift = jnp.zeros_like(k)
        for t in range(ks):
            k_shift = k_shift + k_pad[:, t:t + S, :] * shift_k[:, ks - 1 - t][None, None, :]
        kv = k_shift * v
        L = 2 * S
        kv_pad = jnp.pad(kv, ((0, 0), (0, S), (0, 0)))
        kf_pad = jnp.pad(ssm_k, ((0, 0), (0, S)))
        kv_f = (lambda x, axes=(-2,-1): jnp.fft.rfft2(x.astype(jnp.float32), axes=axes))(kv_pad[:, None, :, :], axes=(1, 2))
        kf_f = (lambda x, axes=(-2,-1): jnp.fft.rfft2(x.astype(jnp.float32), axes=axes))(kf_pad[:, None, :], axes=(1, 2))
        kf_f = (lambda x, *d: x.transpose(*d))(kf_f, 1, 2, 0)
        y_f = kv_f * kf_f[None, :, :, :]
        y = (lambda x, s, axes=(-2,-1): jnp.fft.irfft2(x, s=s, axes=axes).astype(jnp.bfloat16))(y_f, (1, L), axes=(1, 2))[:, 0, :S, :]
        y = y + kv * ssm_D[None, None, :]
        return q * y

    x = A_x
    g = _sigmoid((x * gate_w).sum(-1, keepdims=True))
    a = _A_ref(x, A_wqkv, A_wo)
    b = _B_ref(x, B_k, B_v, B_shift_k, B_ssm_k, B_ssm_D)
    return g * a + (1 - g) * b
```

```python
import math

import numpy as np
import jax
import jax.numpy as jnp
from jax import lax
import jax.experimental.pallas as pl
import jax.experimental.pallas.tpu as pltpu

S = 2048
D = 640
H = 32
DH = D // H
KS = 4

TQ = 512
CK = 128
UNROLL = 4
NQ = S // TQ
NIT = H * NQ
NC = S // CK
K_OFFS = (0, 120, 240, 360, 480, 512)
NG = len(K_OFFS)
VR = 24

BLK = 128
NB = S // BLK
NF = 2 * BLK

F32 = jnp.float32
BF16 = jnp.bfloat16
NT_DIMS = (((1,), (1,)), ((), ()))


def _dft_consts():
    f = np.concatenate([np.arange(0, BLK, 2), np.arange(1, BLK, 2)])
    b = np.arange(BLK)
    th = np.pi * (2 * f[:, None] + 1) * b[None, :] / (2 * BLK)
    fwd = np.concatenate([np.cos(th), -np.sin(th)], axis=0)
    inv = fwd.T / BLK
    return jnp.asarray(fwd, BF16), jnp.asarray(inv, BF16)


def _kernel(x_hbm, w_hbm, wo_hbm, k_hbm, v_hbm, h_hbm, sk_ref, d_ref, gw_ref,
            fwd_ref, inv_ref, out_hbm,
            x_v, w_v, wo_v, k_v, v_v, h_v, out_v,
            wqvt, wkp, kg, qt, vt, ot, s0, s1, qm0, qm1, qm2, qm3, m_ref,
            kpad, kv, uf, hf, zf, sems, osems):
    qm = (qm0, qm1, qm2, qm3)
    sb = (s0, s1)

    cp_w = pltpu.make_async_copy(w_hbm, w_v, sems.at[0])
    cp_x = [pltpu.make_async_copy(x_hbm.at[pl.ds(c * TQ, TQ)], x_v.at[pl.ds(c * TQ, TQ)], sems.at[1 + c])
            for c in range(NQ)]
    cp_k = pltpu.make_async_copy(k_hbm, k_v, sems.at[5])
    cp_v = pltpu.make_async_copy(v_hbm, v_v, sems.at[6])
    cp_h = pltpu.make_async_copy(h_hbm, h_v, sems.at[7])
    cp_wo = pltpu.make_async_copy(wo_hbm, wo_v, sems.at[8])
    cp_w.start()
    cp_x[0].start()
    cp_w.wait()
    for c in range(1, NQ):
        cp_x[c].start()

    with jax.named_scope("wprep"):
        for g, off in enumerate(K_OFFS):
            wkp[:, 128 * g:128 * (g + 1)] = w_v[:, D + off:D + off + 128]
        wqvt[0:D, :] = w_v[:, 0:D].T
        wqvt[D:2 * D, :] = w_v[:, 2 * D:3 * D].T

    qscale = (DH ** -0.5) * math.log2(math.e)
    with jax.named_scope("proj"):
        for c in range(NQ):
            cp_x[c].wait()
            if c == 0:
                cp_k.start()
                cp_v.start()
                cp_h.start()
                cp_wo.start()
            rows = pl.ds(c * TQ, TQ)
            xc = x_v[rows, :]
            kk = jnp.dot(xc, wkp[...], preferred_element_type=F32)
            for g in range(NG):
                kg[g, rows, :] = kk[:, 128 * g:128 * (g + 1)].astype(BF16)
            qv = lax.dot_general(wqvt[...], xc, NT_DIMS, preferred_element_type=F32)
            qt[:, rows] = qv[0:D] * qscale
            sub = lax.broadcasted_iota(jnp.int32, (8, TQ), 0)
            for j in range(H // 2):
                r0 = D + 2 * DH * j
                mid = qv[r0 + 16:r0 + 24]
                vt[2 * j, 0:16, rows] = qv[r0:r0 + 16]
                vt[2 * j, 16:24, rows] = jnp.where(sub < 4, mid, 1.0)
                vt[2 * j + 1, 0:8, rows] = jnp.where(sub < 4, 1.0, mid)
                vt[2 * j + 1, 8:24, rows] = qv[r0 + 24:r0 + 40]

    def grp(i):
        return jnp.minimum((i % H) // 6, NG - 1)

    def build_q(i, qm_ref):
        h = i % H
        qb = i // H
        g = grp(i)
        off = pl.multiple_of(jnp.where(g == NG - 1, K_OFFS[-1], 120 * g), 8)
        q = qt[pl.ds(off, 128), pl.ds(pl.multiple_of(qb * TQ, TQ), TQ)]
        r = lax.broadcasted_iota(jnp.int32, (128, TQ), 0) + off
        lo = h * DH
        qm_ref[...] = jnp.where((r >= lo) & (r < lo + DH), q, 0.0).astype(BF16)

    def step(i, odd, s_nxt, s_cur, qm_ref, m, do_a=True, do_b=True):
        if do_a:
            g = grp(i + 1)
        if do_b:
            h = i % H
            qb = i // H
            acc = jnp.zeros((VR, TQ), F32)
        mx = None
        for c in range(NC):
            ks = pl.ds(c * CK, CK)
            if do_a:
                s = jnp.dot(kg[g, ks, :], qm_ref[...], preferred_element_type=F32)
                s_nxt[ks, :] = s
                cm = jnp.max(s.reshape(CK // 8, 8, TQ), axis=0)
                mx = cm if mx is None else jnp.maximum(mx, cm)
            if do_b:
                sc = s_cur[ks, :].reshape(CK // 8, 8, TQ)
                p = jnp.exp2(sc - m[None]).reshape(CK, TQ).astype(BF16)
                acc = acc + jnp.dot(vt[h, :, ks], p, preferred_element_type=F32)
        if do_b:
            cols = pl.ds(pl.multiple_of(qb * TQ, TQ), TQ)
            pair = h // 2
            if odd:
                o = acc * (1.0 / acc[0:1])
                ot[pair, 20:24, cols] = o[4:8]
                ot[pair, 24:40, cols] = o[8:24]
            else:
                o = acc * (1.0 / acc[20:21])
                ot[pair, 0:16, cols] = o[0:16]
                ot[pair, 16:20, cols] = o[16:20]
        if do_a:
            return jnp.broadcast_to(jnp.max(mx, axis=0, keepdims=True), (8, TQ))
        return None

    def attn_body(j, carry, last=False):
        i0 = UNROLL * j
        m = m_ref[...]
        for u in range(UNROLL):
            i = i0 + u
            do_a = not (last and u == UNROLL - 1)
            if do_a and not (last and u == UNROLL - 2):
                build_q(i + 2, qm[(u + 2) % UNROLL])
            m = step(i, u % 2 == 1, sb[(u + 1) % 2], sb[u % 2], qm[(u + 1) % UNROLL], m, do_a=do_a)
        if not last:
            m_ref[...] = m
        return carry

    with jax.named_scope("attn"):
        build_q(0, qm[0])
        m_ref[...] = step(-1, True, s0, s1, qm[0], None, do_b=False)
        build_q(1, qm[1])
        lax.fori_loop(0, NIT // UNROLL - 1, attn_body, 0)
        attn_body(NIT // UNROLL - 1, 0, last=True)

    cp_k.wait()
    cp_v.wait()
    cp_h.wait()
    cp_wo.wait()
    with jax.named_scope("kv"):
        skf = sk_ref[...].astype(F32)
        kpad[0:8, :] = jnp.zeros((8, D), F32)
        kpad[8:8 + S, :] = k_v[...].astype(F32)

        for a in range(NB):
            r0 = a * BLK
            ksh = kpad[8 + r0:8 + r0 + BLK, :] * skf[0:1]
            for t in range(1, KS):
                ksh = ksh + kpad[8 + r0 - t:8 + r0 - t + BLK, :] * skf[t:t + 1]
            kv[r0:r0 + BLK, :] = ksh * v_v[r0:r0 + BLK, :].astype(F32)

    with jax.named_scope("dft"):
        for a in range(NB):
            r0 = a * BLK
            uf[a] = jnp.dot(fwd_ref[...], kv[r0:r0 + BLK, :].astype(BF16), preferred_element_type=F32)
            zf[a] = lax.dot_general(fwd_ref[...], h_v[:, r0:r0 + BLK], NT_DIMS, preferred_element_type=F32)
        hf[0] = zf[0]
        half = BLK // 2
        for a in range(1, NB):
            hf[a, 0:half] = zf[a, 0:half] - zf[a - 1, BLK:BLK + half]
            hf[a, half:BLK] = zf[a, half:BLK] + zf[a - 1, BLK + half:NF]
            hf[a, BLK:BLK + half] = zf[a, BLK:BLK + half] + zf[a - 1, 0:half]
            hf[a, BLK + half:NF] = zf[a, BLK + half:NF] - zf[a - 1, half:BLK]

    def mac_body(r, carry):
        re = pl.ds(pl.multiple_of(r * 8, 8), 8)
        im = pl.ds(pl.multiple_of(BLK + r * 8, 8), 8)
        for a in range(NB):
            zr = None
            zi = None
            for j in range(a + 1):
                hr = hf[j, re, :]
                hi = hf[j, im, :]
                ur = uf[a - j, re, :]
                ui = uf[a - j, im, :]
                tr = hr * ur - hi * ui
                ti = hr * ui + hi * ur
                zr = tr if zr is None else zr + tr
                zi = ti if zi is None else zi + ti
            zf[a, re, :] = zr
            zf[a, im, :] = zi
        return carry

    with jax.named_scope("mac"):
        lax.fori_loop(0, BLK // 8, mac_body, 0)

    dvec = d_ref[...].astype(F32).reshape(1, D)
    gvec = gw_ref[...].astype(F32).reshape(1, D)
    cp_o = [pltpu.make_async_copy(out_v.at[pl.ds(c * TQ, TQ)], out_hbm.at[pl.ds(c * TQ, TQ)], osems.at[c])
            for c in range(NQ)]
    with jax.named_scope("final"):
        for c in range(NQ):
            cols = pl.ds(c * TQ, TQ)
            o = ot[:, :, cols].reshape(D, TQ).T.astype(BF16)
            att = jnp.dot(o, wo_v[...], preferred_element_type=F32)
            for b in range(TQ // BLK):
                a = c * (TQ // BLK) + b
                rows = pl.ds(a * BLK, BLK)
                y = jnp.dot(inv_ref[...], zf[a].astype(BF16), preferred_element_type=F32)
                xf = x_v[rows, :].astype(F32)
                gate = jax.nn.sigmoid(jnp.sum(xf * gvec, axis=-1, keepdims=True))
                ssm = xf * (y + kv[rows, :] * dvec)
                res = gate * att[b * BLK:(b + 1) * BLK] + (1.0 - gate) * ssm
                out_v[rows, :] = res.astype(BF16)
            cp_o[c].start()
    for c in range(NQ):
        cp_o[c].wait()


@jax.jit
def pallas_gated_mix__mha_block__ssm_conv_h3__prompt_kernel(
    A_x: jax.Array,
    A_wqkv: jax.Array,
    A_wo: jax.Array,
    B_q: jax.Array,
    B_k: jax.Array,
    B_v: jax.Array,
    B_shift_k: jax.Array,
    B_ssm_k: jax.Array,
    B_ssm_D: jax.Array,
    gate_w: jax.Array,
):
    del B_q
    fwd, inv = _dft_consts()
    hbm = pl.BlockSpec(memory_space=pl.ANY)
    vmem = pl.BlockSpec(memory_space=pltpu.VMEM)
    scratch = [
        pltpu.VMEM((S, D), BF16),
        pltpu.VMEM((D, 3 * D), BF16),
        pltpu.VMEM((D, D), BF16),
        pltpu.VMEM((S, D), BF16),
        pltpu.VMEM((S, D), BF16),
        pltpu.VMEM((D, S), BF16),
        pltpu.VMEM((S, D), BF16),
        pltpu.VMEM((2 * D, D), BF16),
        pltpu.VMEM((D, NG * 128), BF16),
        pltpu.VMEM((NG, S, 128), BF16),
        pltpu.VMEM((D, S), F32),
        pltpu.VMEM((H, VR, S), F32),
        pltpu.VMEM((H // 2, 2 * DH, S), F32),
        pltpu.VMEM((S, TQ), F32),
        pltpu.VMEM((S, TQ), F32),
        pltpu.VMEM((128, TQ), BF16),
        pltpu.VMEM((128, TQ), BF16),
        pltpu.VMEM((128, TQ), BF16),
        pltpu.VMEM((128, TQ), BF16),
        pltpu.VMEM((8, TQ), F32),
        pltpu.VMEM((S + 8, D), F32),
        pltpu.VMEM((S, D), F32),
        pltpu.VMEM((NB, NF, D), F32),
        pltpu.VMEM((NB, NF, D), F32),
        pltpu.VMEM((NB, NF, D), F32),
        pltpu.SemaphoreType.DMA((9,)),
        pltpu.SemaphoreType.DMA((NQ,)),
    ]
    out = pl.pallas_call(
        _kernel,
        out_shape=jax.ShapeDtypeStruct((S, D), BF16),
        in_specs=[hbm] * 6 + [vmem] * 5,
        out_specs=hbm,
        scratch_shapes=scratch,
        compiler_params=pltpu.CompilerParams(vmem_limit_bytes=120 * 1024 * 1024),
        name="gated_mix_mha_h3",
    )(A_x.reshape(S, D), A_wqkv, A_wo, B_k.reshape(S, D), B_v.reshape(S, D), B_ssm_k,
      B_shift_k.T, B_ssm_D, gate_w, fwd, inv)
    return out.reshape(1, S, D)
```

```python
import math

import numpy as np
import jax
import jax.numpy as jnp
from jax import lax
import jax.experimental.pallas as pl
import jax.experimental.pallas.tpu as pltpu

S = 2048
D = 640
H = 32
DH = D // H
KS = 4
LT = D // 128

TQ = 512
CK = 128
NQ = S // TQ
NIT = H * NQ
NC = S // CK
UNROLL = 8
K_OFFS = (0, 120, 240, 360, 480, 512)
NG = len(K_OFFS)
VR = 24

BLK = 128
NB = S // BLK
NF = 2 * BLK
NR = BLK // 8
BPC = TQ // BLK
SPEC_ROWS = 3 * NB * 16 + 128
KV_ROWS = 32
MAC_TOK = 4

F32 = jnp.float32
BF16 = jnp.bfloat16
U32 = jnp.uint32
NT_DIMS = (((1,), (1,)), ((), ()))

assert NIT // UNROLL == NR


def _dft_consts():
    f = np.concatenate([np.arange(0, BLK, 2), np.arange(1, BLK, 2)])
    b = np.arange(BLK)
    th = np.pi * (2 * f[:, None] + 1) * b[None, :] / (2 * BLK)
    re = np.cos(th).reshape(NR, 8, BLK)
    im = (-np.sin(th)).reshape(NR, 8, BLK)
    fwd = np.concatenate([re, im], axis=1).reshape(NF, BLK)
    inv = fwd.T / BLK
    return jnp.asarray(fwd, BF16), jnp.asarray(inv, BF16)


def _kernel(z_ref, x_hbm, w_hbm, wo_hbm, k_hbm, v_hbm, h_hbm, sk_ref, d_ref, gw_ref,
            fwd_ref, inv_ref, out_hbm,
            x_v, w_v, wo_v, k_v, v_v, h_v, out_v,
            kg, qt, vt, ot, s0, s1, m_ref, kv, hprev, spec,
            qm0, qm1, qm2, qm3, qm4, qm5, qm6, qm7,
            sems, osems):
    qm = (qm0, qm1, qm2, qm3, qm4, qm5, qm6, qm7)
    sb = (s0, s1)
    z8 = pl.multiple_of(z_ref[0] * 128, 128)
    zt = z_ref[1]

    def rows_cp(src, dst, c, sem):
        return pltpu.make_async_copy(src.at[pl.ds(c * TQ, TQ)], dst.at[pl.ds(c * TQ, TQ)], sem)

    def cp_x(c):
        return rows_cp(x_hbm, x_v, c, sems.at[0, c])

    def cp_k(c):
        return rows_cp(k_hbm, k_v, c, sems.at[1, c])

    def cp_v(c):
        return rows_cp(v_hbm, v_v, c, sems.at[2, c])

    def cp_h(c):
        return pltpu.make_async_copy(h_hbm.at[:, pl.ds(c * TQ, TQ)], h_v.at[c], sems.at[3, c])

    cp_w = pltpu.make_async_copy(w_hbm, w_v, sems.at[4, 0])
    cp_wo = pltpu.make_async_copy(wo_hbm, wo_v, sems.at[4, 1])
    cp_w.start()
    cp_x(0).start()
    s1[...] = jnp.zeros((S, TQ), F32)
    m_ref[...] = jnp.zeros((8, TQ), F32)
    hprev[...] = jnp.zeros((NF, D), F32)
    cp_w.wait()
    for c in range(NQ):
        if c > 0:
            cp_x(c).start()
        cp_k(c).start()
        cp_v(c).start()
        cp_h(c).start()
    cp_wo.start()

    qscale = (DH ** -0.5) * math.log2(math.e)

    def proj_body(c, carry):
        r0 = pl.multiple_of(c * TQ, TQ)
        rows = pl.ds(r0, TQ)
        cp_x(c).wait()
        xc = x_v[rows, :]
        q = jnp.dot(xc, w_v[:, 0:D], preferred_element_type=F32)

        cp_k(c).wait()
        cp_v(c).wait()
        cp_h(c).wait()
        qt[:, rows] = (q * qscale).T
        xc = x_v[rows, :]
        vv = jnp.dot(xc, w_v[:, 2 * D:3 * D], preferred_element_type=F32)
        kk = jnp.dot(xc, w_v[:, D:2 * D], preferred_element_type=F32)
        vtr = vv.T
        sub = lax.broadcasted_iota(jnp.int32, (8, TQ), 0)
        for j in range(H // 2):
            b0 = 2 * DH * j
            mid = vtr[b0 + 16:b0 + 24]
            vt[2 * j, 0:16, rows] = vtr[b0:b0 + 16]
            vt[2 * j, 16:24, rows] = jnp.where(sub < 4, mid, 1.0)
            vt[2 * j + 1, 0:8, rows] = jnp.where(sub < 4, 1.0, mid)
            vt[2 * j + 1, 8:24, rows] = vtr[b0 + 24:b0 + 40]
        r0h = pl.multiple_of(c * (TQ // 2), TQ // 2)
        for g, off in enumerate(K_OFFS):
            kg[g, pl.ds(r0h, TQ // 2), :] = pltpu.bitcast(kk[:, off:off + 128].astype(BF16), U32)

        skf = sk_ref[...].astype(F32)
        pr = KV_ROWS
        npc = (TQ // pr) * LT
        per_tile = npc // (2 * LT)
        for n in range(npc):
            p, lt = divmod(n, LT)
            ls = slice(lt * 128, (lt + 1) * 128)
            tile, tr = divmod(n, per_tile)
            src = vv if tile < LT else kk
            tr0 = tr * (TQ // per_tile)
            tl0 = (tile % LT) * 128
            k_v[pl.ds(pl.multiple_of(S + zt * 16, 16), 16), 0:128] = pltpu.bitcast(
                src[tr0:tr0 + 8, tl0:tl0 + 128], BF16)
            p0 = pl.multiple_of(r0 + p * pr, pr)
            cur = k_v[pl.ds(p0, pr), ls].astype(F32)
            prev = k_v[pl.ds(pl.multiple_of(jnp.maximum(p0 - 16, 0), 16), 16), ls].astype(F32)[8:16]
            if p == 0:
                prev = jnp.where(c > 0, prev, 0.0)
            ext = jnp.concatenate([prev, cur], axis=0)
            ksh = cur * skf[0:1, ls]
            for t in range(1, KS):
                ksh = ksh + ext[8 - t:8 - t + pr] * skf[t:t + 1, ls]
            kv[pl.ds(p0, pr), ls] = ksh * v_v[pl.ds(p0, pr), ls].astype(F32)

        hp = hprev[...].reshape(NR, 16, D)
        for b in range(BPC):
            a16 = pl.multiple_of((c * BPC + b) * 16, 16)
            hraw = lax.dot_general(fwd_ref[...], h_v[c, :, b * BLK:(b + 1) * BLK], NT_DIMS,
                                   preferred_element_type=F32).reshape(NR, 16, D)
            e = NR // 2
            hre = jnp.concatenate([hraw[:e, 0:8] - hp[:e, 8:16], hraw[e:, 0:8] + hp[e:, 8:16]], axis=0)
            him = jnp.concatenate([hraw[:e, 8:16] + hp[:e, 0:8], hraw[e:, 8:16] - hp[e:, 0:8]], axis=0)
            for lt in range(LT):
                ls = slice(lt * 128, (lt + 1) * 128)
                spec[:, lt, pl.ds(NB * 16 + a16, 8), :] = hre[:, :, ls]
                spec[:, lt, pl.ds(NB * 16 + a16 + 8, 8), :] = him[:, :, ls]
            hp = hraw
        hprev[...] = hp.reshape(NF, D)
        for b in range(BPC):
            a16 = pl.multiple_of((c * BPC + b) * 16, 16)
            ub = kv[pl.ds(pl.multiple_of(r0 + b * BLK, BLK), BLK), :]
            uf = jnp.dot(fwd_ref[...], ub.astype(BF16), preferred_element_type=F32).reshape(NR, 16, D)
            for lt in range(LT):
                spec[:, lt, pl.ds(a16, 16), :] = uf[:, :, lt * 128:(lt + 1) * 128]
        return carry

    with jax.named_scope("proj"):
        lax.fori_loop(0, NQ, proj_body, 0)

    def grp(h):
        return jnp.minimum(h // 6, NG - 1)

    def build_q(i, qm_ref):
        i = jnp.minimum(i, NIT - 1)
        h = i // NQ
        qb = i % NQ
        g = grp(h)
        off = pl.multiple_of(jnp.where(g == NG - 1, K_OFFS[-1], 120 * g), 8)
        q = qt[pl.ds(off, 128), pl.ds(pl.multiple_of(qb * TQ, TQ), TQ)]
        r = lax.broadcasted_iota(jnp.int32, (128, TQ), 0) + off
        lo = h * DH
        q = jnp.where((r >= lo) & (r < lo + DH), q, 0.0)
        qm_ref[pl.ds(z8, 64), :] = pltpu.bitcast(q.astype(BF16), U32)

    class SpecMac:
        def __init__(self, r):
            self.r = r
            self.items = [(lt, a, j) for lt in range(LT) for a in range(NB) for j in range(a + 1)]
            self.pos = 0
            self.zr = None
            self.zi = None

        def run(self, n):
            r = self.r
            for lt, a, j in self.items[self.pos:self.pos + n]:
                hb = (NB + j) * 16
                ub = (a - j) * 16
                hr = spec[r, lt, hb:hb + 8, :]
                hi = spec[r, lt, hb + 8:hb + 16, :]
                ur = spec[r, lt, ub:ub + 8, :]
                ui = spec[r, lt, ub + 8:ub + 16, :]
                tr = hr * ur - hi * ui
                ti = hr * ui + hi * ur
                self.zr = tr if j == 0 else self.zr + tr
                self.zi = ti if j == 0 else self.zi + ti
                if j == a:
                    zb = (2 * NB + a) * 16
                    spec[r, lt, zb:zb + 8, :] = self.zr
                    spec[r, lt, zb + 8:zb + 16, :] = self.zi
            self.pos += n

    mac_per_tok = -(-(LT * NB * (NB + 1) // 2) // (UNROLL * (NC - 2) * MAC_TOK))

    def step(i, odd_b, s_a, s_b, qm_ref, m, mac, do_a=True):
        if do_a:
            g = grp(i // NQ)
        ib = i - 1
        hb = jnp.where(ib < 0, 1, ib // NQ)
        pair = jnp.where(ib < 0, H // 2, hb // 2)
        cols = pl.ds(pl.multiple_of((ib % NQ) * TQ, TQ), TQ)
        acc = jnp.zeros((VR, TQ), F32)
        mx = None
        for c in range(NC):
            if do_a:
                kc = pltpu.bitcast(kg[g, pl.ds(c * CK // 2, CK // 2), :], BF16)
                s = jnp.dot(kc, pltpu.bitcast(qm_ref[pl.ds(z8, 64), :], BF16), preferred_element_type=F32)
                s_a[pl.ds(c * CK + z8, CK), :] = s
                cm = jnp.max(s.reshape(CK // 8, 8, TQ), axis=0)
                mx = cm if mx is None else jnp.maximum(mx, cm)
                if 1 <= c <= NC - 2:
                    for t in range(MAC_TOK):
                        tk = t * CK // MAC_TOK
                        spec[zt, 0, SPEC_ROWS - 8:SPEC_ROWS, :] = s[tk:tk + 8, 128:256]
                        mac.run(mac_per_tok)
            sc = s_b[pl.ds(c * CK + z8, CK), :].reshape(CK // 8, 8, TQ)
            p = jnp.exp2(sc - m[None]).reshape(CK, TQ).astype(BF16)
            acc = acc + jnp.dot(vt[hb, :, pl.ds(c * CK, CK)], p, preferred_element_type=F32)
        if odd_b:
            o = acc * (1.0 / acc[0:1])
            ot[pair, 20:24, cols] = o[4:8]
            ot[pair, 24:40, cols] = o[8:24]
        else:
            o = acc * (1.0 / acc[20:21])
            ot[pair, 0:16, cols] = o[0:16]
            ot[pair, 16:20, cols] = o[16:20]
        if do_a:
            return jnp.broadcast_to(jnp.max(mx, axis=0, keepdims=True), (8, TQ))
        return None

    def attn_body(j, carry):
        m = m_ref[...]
        mac = SpecMac(j)
        for u in range(UNROLL):
            i = UNROLL * j + u
            build_q(i + 1, qm[(u + 1) % UNROLL])
            odd_b = ((u - 1) // NQ) % 2 == 1
            m = step(i, odd_b, sb[u % 2], sb[(u + 1) % 2], qm[u], m, mac)
        assert mac.pos >= len(mac.items)
        m_ref[...] = m
        return carry

    with jax.named_scope("attn"):
        build_q(0, qm[0])
        lax.fori_loop(0, NIT // UNROLL, attn_body, 0)
        step(NIT, True, None, s1, None, m_ref[...], None, do_a=False)

    cp_wo.wait()

    def cp_o(c):
        return rows_cp(out_v, out_hbm, c, osems.at[c])

    def final_body(c, carry):
        dvec = d_ref[...].astype(F32).reshape(1, D)
        gvec = gw_ref[...].astype(F32).reshape(1, D)
        r0 = pl.multiple_of(c * TQ, TQ)
        ys = []
        for b in range(BPC):
            z16 = pl.multiple_of((2 * NB + c * BPC + b) * 16, 16)
            zz = jnp.concatenate([spec[:, lt, pl.ds(z16, 16), :].reshape(NF, 128) for lt in range(LT)], axis=1)
            ys.append(jnp.dot(inv_ref[...], zz.astype(BF16), preferred_element_type=F32))
        for b in range(BPC):
            rows = pl.ds(pl.multiple_of(r0 + b * BLK, BLK), BLK)
            o = ot[0:H // 2, :, rows].reshape(D, BLK).T.astype(BF16)
            att = jnp.dot(o, wo_v[...], preferred_element_type=F32)
            xf = x_v[rows, :].astype(F32)
            gate = jax.nn.sigmoid(jnp.sum(xf * gvec, axis=-1, keepdims=True))
            ssm = xf * (ys[b] + kv[rows, :] * dvec)
            out_v[rows, :] = (gate * att + (1.0 - gate) * ssm).astype(BF16)
        cp_o(c).start()
        return carry

    with jax.named_scope("final"):
        lax.fori_loop(0, NQ, final_body, 0)
    for c in range(NQ):
        cp_o(c).wait()


@jax.jit
def pallas_gated_mix__mha_block__ssm_conv_h3__prompt_kernel(
    A_x: jax.Array,
    A_wqkv: jax.Array,
    A_wo: jax.Array,
    B_q: jax.Array,
    B_k: jax.Array,
    B_v: jax.Array,
    B_shift_k: jax.Array,
    B_ssm_k: jax.Array,
    B_ssm_D: jax.Array,
    gate_w: jax.Array,
):
    del B_q
    fwd, inv = _dft_consts()
    zeros = jnp.asarray(np.zeros((2,), np.int32))
    hbm = pl.BlockSpec(memory_space=pl.ANY)
    vmem = pl.BlockSpec(memory_space=pltpu.VMEM)
    smem = pl.BlockSpec(memory_space=pltpu.SMEM)
    scratch = [
        pltpu.VMEM((S, D), BF16),
        pltpu.VMEM((D, 3 * D), BF16),
        pltpu.VMEM((D, D), BF16),
        pltpu.VMEM((S + 16, D), BF16),
        pltpu.VMEM((S, D), BF16),
        pltpu.VMEM((NQ, D, TQ), BF16),
        pltpu.VMEM((S, D), BF16),
        pltpu.VMEM((NG, S // 2, 128), U32),
        pltpu.VMEM((D, S), F32),
        pltpu.VMEM((H, VR, S), F32),
        pltpu.VMEM((H // 2 + 1, 2 * DH, S), F32),
        pltpu.VMEM((S, TQ), F32),
        pltpu.VMEM((S, TQ), F32),
        pltpu.VMEM((8, TQ), F32),
        pltpu.VMEM((S, D), F32),
        pltpu.VMEM((NF, D), F32),
        pltpu.VMEM((NR, LT, SPEC_ROWS, 128), F32),
    ] + [pltpu.VMEM((64, TQ), U32)] * UNROLL + [
        pltpu.SemaphoreType.DMA((5, NQ)),
        pltpu.SemaphoreType.DMA((NQ,)),
    ]
    out = pl.pallas_call(
        _kernel,
        out_shape=jax.ShapeDtypeStruct((S, D), BF16),
        in_specs=[smem] + [hbm] * 6 + [vmem] * 5,
        out_specs=hbm,
        scratch_shapes=scratch,
        compiler_params=pltpu.CompilerParams(vmem_limit_bytes=120 * 1024 * 1024),
        name="gated_mix_mha_h3",
    )(zeros, A_x.reshape(S, D), A_wqkv, A_wo, B_k.reshape(S, D), B_v.reshape(S, D), B_ssm_k,
      B_shift_k.T, B_ssm_D, gate_w, fwd, inv)
    return out.reshape(1, S, D)
```

```python
import math

import numpy as np
import jax
import jax.numpy as jnp
from jax import lax
import jax.experimental.pallas as pl
import jax.experimental.pallas.tpu as pltpu

S = 2048
D = 640
H = 32
DH = D // H
KS = 4
LT = D // 128

TQ = 512
QL = TQ // 128
CK = 128
NQ = S // TQ
NIT = H * NQ
NC = S // CK
NP = H // 2
UNROLL = 2 * NQ
WL = 2 * DH
KD = 48
VR = 24

GK = 16
GM = CK // GK - 1
NV = NC * GK
KR = NP * (S // 2)
VTR = NP * NC * VR
KB_SETS = 4
KB_PIECES = DH * KB_SETS
KB_SLOTS = 46
REF_SLOT = 4
REF_OFF = 32.0
DEN_LO = 2.0 ** -48
DEN_HI = 2.0 ** 100
OUT_HI = 2.0 ** 126

BLK = 128
NB = S // BLK
NF = 2 * BLK
NR = BLK // 8
BPC = TQ // BLK
KV_ROWS = 32
KV_TILES = 8
MAC_TOK = 2

F32 = jnp.float32
BF16 = jnp.bfloat16
U32 = jnp.uint32
NT_DIMS = (((1,), (1,)), ((), ()))

assert NP == NR and BPC * CK == TQ


def _dft_consts():
    f = np.concatenate([np.arange(0, BLK, 2), np.arange(1, BLK, 2)])
    b = np.arange(BLK)
    th = np.pi * (2 * f[:, None] + 1) * b[None, :] / (2 * BLK)
    re = np.cos(th).reshape(NR, 8, BLK)
    im = (-np.sin(th)).reshape(NR, 8, BLK)
    fwd = np.concatenate([re, im], axis=1).reshape(NF, BLK)
    inv = fwd.T / BLK
    return jnp.asarray(fwd, BF16), jnp.asarray(inv, BF16)


def _kb_pos(slot):
    return min(KB_PIECES, KB_PIECES * max(slot - 1, 0) // KB_SLOTS)


def _lanes(l):
    return slice(l * 128, (l + 1) * 128)


def _kernel(z_hbm, x_hbm, w_hbm, wo_hbm, k_hbm, v_hbm, h_hbm, sk_hbm, d_hbm, gw_hbm,
            fwd_hbm, inv_hbm, out_hbm,
            qm, qs, vp0, vp1, kb0, kb1, kf, uh, zo, pcar, wt0, wt1,
            kv, hprev, x_v, v_v, h_v, out_v, ot, k_v, w_v, wo_v, m_ref, acc_ref, bad_ref,
            fwd_ref, inv_ref, sk_ref, d_ref, gw_ref, z_ref, redo_ref, sems, osems):
    vps = (vp0, vp1)
    kbs = (kb0, kb1)
    wts = (wt0, wt1)

    def rows_cp(src, dst, c, sem):
        return pltpu.make_async_copy(src.at[pl.ds(c * TQ, TQ)], dst.at[pl.ds(c * TQ, TQ)], sem)

    def cp_x(c):
        return rows_cp(x_hbm, x_v, c, sems.at[0, c])

    def cp_k(c):
        return rows_cp(k_hbm, k_v, c, sems.at[1, c])

    def cp_v(c):
        return rows_cp(v_hbm, v_v, c, sems.at[2, c])

    def cp_h(c):
        return pltpu.make_async_copy(h_hbm.at[:, pl.ds(c * TQ, TQ)], h_v.at[c], sems.at[3, c])

    def cp_w(n):
        return pltpu.make_async_copy(w_hbm.at[:, pl.ds(n * D, D)], w_v.at[n], sems.at[4, n])

    cp_wo = pltpu.make_async_copy(wo_hbm, wo_v, sems.at[4, 3])
    small = [pltpu.make_async_copy(src, dst, sems.at[5 + n // NQ, n % NQ]) for n, (src, dst) in enumerate(
        [(z_hbm, z_ref), (fwd_hbm, fwd_ref), (sk_hbm, sk_ref), (inv_hbm, inv_ref), (d_hbm, d_ref),
         (gw_hbm, gw_ref)])]
    cp_w(0).start()
    for c in range(NQ):
        cp_x(c).start()
    for cp in small:
        cp.start()
    cp_w(1).start()
    cp_w(2).start()
    for c in range(NQ):
        cp_k(c).start()
        cp_v(c).start()
        cp_h(c).start()
    cp_wo.start()
    hprev[...] = jnp.zeros((NF, D), F32)
    pcar[...] = jnp.zeros((CK // 2, TQ), U32)
    acc_ref[...] = jnp.ones((VR, TQ), F32)
    bad_ref[...] = jnp.zeros((8, BLK), F32)
    cp_w(0).wait()

    qscale = (DH ** -0.5) * math.log2(math.e)

    def qproj_body(c, carry):
        cp_x(c).wait()
        xc = x_v[pl.ds(pl.multiple_of(c * TQ, TQ), TQ), :]
        q = jnp.dot(xc, w_v[0], preferred_element_type=F32)
        qtr = (q * qscale).T
        low = lax.broadcasted_iota(jnp.int32, (8, TQ), 0) < 4
        zero8 = jnp.zeros((8, TQ), F32)
        for h in range(H):
            s0 = (h * DH // 8) * 8
            qs[h * NQ + c, 0:VR, :] = qtr[s0:s0 + VR]
            b0 = (h // 2) * WL
            mid = qtr[b0 + 16:b0 + 24]
            if h % 2 == 0:
                wrows = [qtr[b0:b0 + 16], jnp.where(low, mid, 0.0), zero8, zero8, zero8]
            else:
                wrows = [zero8, zero8, jnp.where(low, 0.0, mid), qtr[b0 + 24:b0 + 40], zero8]
            qm[h * NQ + c, 0:KD // 2, :] = pltpu.bitcast(jnp.concatenate(wrows, axis=0).astype(BF16), U32)
        return carry

    lax.fori_loop(0, NQ, qproj_body, 0)

    for cp in small:
        cp.wait()
    cp_w(1).wait()
    cp_w(2).wait()
    zt = z_ref[0]
    kb_tok = pl.ds(pl.multiple_of(VTR + NV * DH + zt * 8, 8), 8)
    vp_tok = pl.ds(pl.multiple_of(KR + QL * NV + zt * 8, 8), 8)
    kv_tok = pl.ds(pl.multiple_of(S + zt * 16, 16), 16)
    wt_rows = pl.ds(pl.multiple_of(zt * 128, 128), 8)
    zo_tok = NR + zt
    ot_tok = H + 1 + zt

    def window(src, j):
        t, off = divmod(j * WL, 128)
        w = src[:, _lanes(t)]
        if off:
            w = pltpu.roll(w, 128 - off, axis=1)
        if off + WL > 128:
            ln = lax.broadcasted_iota(jnp.int32, w.shape, 1)
            w = jnp.where(ln < 128 - off, w, pltpu.roll(src[:, _lanes(t + 1)], 128 - off, axis=1))
        return w

    def proj_body(c, carry):
        r0 = pl.multiple_of(c * TQ, TQ)
        cp_k(c).wait()
        cp_v(c).wait()
        cp_h(c).wait()

        hp = hprev[...].reshape(NR, 16, D)
        for b in range(BPC):
            a16 = pl.multiple_of((c * BPC + b) * 16, 16)
            hraw = lax.dot_general(fwd_ref[...], h_v[c, :, b * BLK:(b + 1) * BLK], NT_DIMS,
                                   preferred_element_type=F32).reshape(NR, 16, D)
            e = NR // 2
            hre = jnp.concatenate([hraw[:e, 0:8] - hp[:e, 8:16], hraw[e:, 0:8] + hp[e:, 8:16]], axis=0)
            him = jnp.concatenate([hraw[:e, 8:16] + hp[:e, 0:8], hraw[e:, 8:16] - hp[e:, 0:8]], axis=0)
            for lt in range(LT):
                uh[:, lt, pl.ds(NB * 16 + a16, 8), :] = hre[:, :, _lanes(lt)]
                uh[:, lt, pl.ds(NB * 16 + a16 + 8, 8), :] = him[:, :, _lanes(lt)]
            hp = hraw
        hprev[...] = hp.reshape(NF, D)

        xc = x_v[pl.ds(r0, TQ), :]
        kk = jnp.dot(xc, w_v[1], preferred_element_type=F32)
        vv = jnp.dot(xc, w_v[2], preferred_element_type=F32)

        ksel = jnp.concatenate([kk[(b + 1) * CK - GK:(b + 1) * CK] for b in range(BPC)], axis=0)
        kcol = []
        for b in range(BPC):
            kcol.append([jnp.broadcast_to(ksel[b * GK:(b + 1) * GK, d:d + 1], (GK, 128)) for d in range(DH)])
            t0 = pl.multiple_of(VTR + (c * BPC + b) * (GK * DH), GK)
            kb0[pl.ds(t0, DH * GK), :] = jnp.concatenate(kcol[b], axis=0)

        lane = lax.broadcasted_iota(jnp.int32, (TQ // 2, 128), 1)
        ones_l = jnp.where(lane < WL + 2, jnp.uint32(0x3F803F80), jnp.uint32(0))
        r0h = pl.multiple_of(c * (TQ // 2), TQ // 2)
        kkb = pltpu.bitcast(kk.astype(BF16), U32)
        for j in range(NP):
            kw = jnp.where(lane < WL, window(kkb, j), ones_l)
            vp0[pl.ds(j * (S // 2) + r0h, TQ // 2), :] = kw
            vp1[pl.ds(j * (S // 2) + r0h, TQ // 2), :] = kw
            kf[j, pl.ds(pl.multiple_of(c * (BPC * GK), GK), BPC * GK), :] = window(ksel, j)

        for b in range(BPC):
            g0 = pl.multiple_of((c * BPC + b) * GK, GK)
            for l in range(QL):
                sv = None
                for d in range(DH):
                    t = kcol[b][d] * qs[0, d:d + 1, _lanes(l)]
                    sv = t if sv is None else sv + t
                vp0[pl.ds(KR + l * NV + g0, GK), :] = pltpu.bitcast(sv, U32)

        low = lax.broadcasted_iota(jnp.int32, (8, TQ), 0) < 4
        vtr = vv.T
        for j in range(NP):
            b0 = j * WL
            mid = vtr[b0 + 16:b0 + 24]
            slabs = (jnp.concatenate([vtr[b0:b0 + 16], jnp.where(low, mid, 1.0)], axis=0),
                     jnp.concatenate([jnp.where(low, 1.0, mid), vtr[b0 + 24:b0 + 40]], axis=0))
            for par in range(2):
                for b in range(BPC):
                    vr0 = pl.multiple_of((j * NC + c * BPC + b) * VR, 8)
                    kbs[1 - par][pl.ds(vr0, VR), :] = slabs[par][:, b * CK:(b + 1) * CK]

        skf = sk_ref[...].astype(F32)
        npc = (TQ // KV_ROWS) * LT
        per_tile = npc // KV_TILES
        for n in range(npc):
            p, lt = divmod(n, LT)
            ls = _lanes(lt)
            tile, tr = divmod(n, per_tile)
            tr0 = (tr * (TQ // 8) // per_tile) * 8
            src = kk if tile < LT else vv
            k_v[kv_tok, 0:128] = pltpu.bitcast(src[tr0:tr0 + 8, _lanes(tile % LT)], BF16)
            p0 = pl.multiple_of(r0 + p * KV_ROWS, KV_ROWS)
            cur = k_v[pl.ds(p0, KV_ROWS), ls].astype(F32)
            prev = k_v[pl.ds(pl.multiple_of(jnp.maximum(p0 - 16, 0), 16), 16), ls].astype(F32)[8:16]
            if p == 0:
                prev = jnp.where(c > 0, prev, 0.0)
            ext = jnp.concatenate([prev, cur], axis=0)
            ksh = cur * skf[0:1, ls]
            for t in range(1, KS):
                ksh = ksh + ext[8 - t:8 - t + KV_ROWS] * skf[t:t + 1, ls]
            kv[pl.ds(p0, KV_ROWS), ls] = ksh * v_v[pl.ds(p0, KV_ROWS), ls].astype(F32)

        for b in range(BPC):
            a16 = pl.multiple_of((c * BPC + b) * 16, 16)
            ub = kv[pl.ds(pl.multiple_of(r0 + b * BLK, BLK), BLK), :]
            uf = jnp.dot(fwd_ref[...], ub.astype(BF16), preferred_element_type=F32).reshape(NR, 16, D)
            for lt in range(LT):
                uh[:, lt, pl.ds(a16, 16), :] = uf[:, :, _lanes(lt)]
        return carry

    lax.fori_loop(0, NQ, proj_body, 0)

    def build_kb(pair, par, piece, tok):
        d, q = divmod(piece, KB_SETS)
        n = NV // KB_SETS
        ln = par * DH + d
        val = jnp.broadcast_to(kf[pair, q * n:(q + 1) * n, ln:ln + 1], (n, 128))
        kbs[par][kb_tok, :] = tok
        for k in range(n // GK):
            g = q * (n // GK) + k
            kbs[par][pl.ds(VTR + (g * DH + d) * GK, GK), :] = val[k * GK:(k + 1) * GK]

    class SpecMac:
        def __init__(self, r):
            self.r = r
            self.items = [(lt, a, j) for lt in range(LT) for a in range(NB) for j in range(a + 1)]
            self.per = -(-len(self.items) // ((UNROLL * NC - 2) * MAC_TOK))
            self.pos = 0
            self.zr = None
            self.zi = None

        def run(self, tok):
            r = self.r
            for lt, a, j in self.items[self.pos:self.pos + self.per]:
                hb = (NB + j) * 16
                ub = (a - j) * 16
                hr = uh[r, lt, hb:hb + 8, :]
                hi = uh[r, lt, hb + 8:hb + 16, :]
                ur = uh[r, lt, ub:ub + 8, :]
                ui = uh[r, lt, ub + 8:ub + 16, :]
                tr = hr * ur - hi * ui
                ti = hr * ui + hi * ur
                self.zr = tr if j == 0 else self.zr + tr
                self.zi = ti if j == 0 else self.zi + ti
                if j == a:
                    zo[zo_tok, 0, 0:8, :] = tok
                    zo[r, lt, a * 16:a * 16 + 8, :] = self.zr
                    zo[r, lt, a * 16 + 8:a * 16 + 16, :] = self.zi
            self.pos += self.per

    class Step:
        def __init__(self, u, i):
            self.par = (u // NQ) % 2
            self.buf = vps[u % 2]
            self.wt = wts[u % 2]
            self.i = i
            self.pos = 0

        def vpu_piece(self, tok):
            g, l = self.pos % NC, (self.pos + self.pos // NC) % QL
            self.pos += 1
            sv = [None, None]
            for d in range(DH):
                qr = 4 * self.par + d
                t = kbs[self.par][pl.ds(VTR + (g * DH + d) * GK, GK), :] * qs[self.i, qr:qr + 1, _lanes(l)]
                sv[d % 2] = t if d < 2 else sv[d % 2] + t
            if tok is not None:
                self.buf[vp_tok, :] = pltpu.bitcast(tok, U32)
            self.buf[pl.ds(KR + l * NV + g * GK, GK), :] = pltpu.bitcast(sv[0] + sv[1], U32)

        def vpu_scores(self, groups):
            return jnp.concatenate(
                [pltpu.bitcast(self.buf[pl.ds(KR + l * NV + groups[l] * GK, GK), :], F32) for l in range(QL)],
                axis=1).reshape(GK // 8, 8, TQ)

        def set_reference(self):
            mx = jnp.max(jnp.max(self.vpu_scores(range(QL)), axis=0), axis=0, keepdims=True)
            mb = jnp.broadcast_to((mx + REF_OFF).astype(BF16).astype(F32), (8, TQ))
            sub = lax.broadcasted_iota(jnp.int32, (8, TQ), 0)
            self.wt[wt_rows, :] = jnp.where(sub == WL // 2 - 16, pltpu.bitcast(-mb, U32), qm[self.i, 16:24, :])
            return mb

        def weights(self):
            return pltpu.bitcast(jnp.concatenate([qm[self.i, 0:16, :], self.wt[wt_rows, :]], axis=0), BF16)

    def pv_tile(vrow, head, par, qb, t, p, acc):
        pv = jnp.dot(kbs[1 - par][pl.ds(vrow + t * VR, VR), :], p, preferred_element_type=F32)
        acc = pv if t == 0 else pv + acc
        if t == NC - 1:
            ot[head, :, qb * TQ:(qb + 1) * TQ] = acc
        return acc

    def attn_body(j, carry):
        i0 = UNROLL * j
        m = m_ref[...]
        acc = acc_ref[...]
        mac = SpecMac(j)
        krow = pl.multiple_of(j * (S // 2), S // 2)
        vrow = pl.multiple_of(j * (NC * VR), NC * VR)
        vrow_prev = pl.multiple_of(jnp.maximum(j - 1, 0) * (NC * VR), NC * VR)
        pair_next = jnp.minimum(j + 1, NP - 1)
        pend = (vrow_prev, jnp.where(j > 0, 2 * j - 1, H), 1, NQ - 1, NC - 1, pltpu.bitcast(pcar[...], BF16))
        sprev = None
        sprev2 = None
        nxt = Step(0, i0)
        for u in range(UNROLL):
            last = u == UNROLL - 1
            head = 2 * j + u // NQ
            cur = nxt
            nxt = Step(u + 1, jnp.minimum(i0 + u + 1, NIT - 1) if last else i0 + u + 1)
            kbuf = cur.buf if last else nxt.buf
            for c in range(NC):
                parts = []
                for t in range(QL):
                    p1 = GM * (t + 1) // QL
                    for pp in range(GM * t // QL, p1):
                        key0 = c * CK + GK * (GM - 1 - pp)
                        parts.append(kbuf[pl.ds(krow + key0 // 2, GK // 2), 0:KD])
                    jj, src = (2 * p1 - 4, sprev) if p1 >= 2 else (2 * GM - 1, sprev2)
                    nxt.vpu_piece(None if src is None else src[jj * 8:jj * 8 + 8, 0:128])
                kc = pltpu.bitcast(jnp.concatenate(parts, axis=0), BF16)
                s = jnp.dot(kc, cur.weights(), preferred_element_type=F32)
                pe = jnp.exp2(s)
                acc = pv_tile(*pend, acc)
                tile = [pe[pp * GK:(pp + 1) * GK] for pp in range(GM - 1, -1, -1)]
                tile.append(jnp.exp2(cur.vpu_scores([c] * QL) - m[None]).reshape(GK, TQ))
                pend = (vrow, head, cur.par, u % NQ, c, jnp.concatenate(tile, axis=0))
                if c == REF_SLOT:
                    m_next = nxt.set_reference()
                slot = (u % NQ) * NC + c
                for piece in range(_kb_pos(slot), _kb_pos(slot + 1)):
                    jj = (piece - _kb_pos(slot)) * 6 + 1
                    build_kb(pair_next if cur.par else j, 1 - cur.par, piece, s[jj * 8:jj * 8 + 8, 256:384])
                for t in range(MAC_TOK):
                    jj = t * 2 * GM // MAC_TOK
                    mac.run(s[jj * 8:jj * 8 + 8, 128:256])
                sprev2 = sprev
                sprev = s
            m = m_next
        assert mac.pos >= len(mac.items)
        m_ref[...] = m
        acc_ref[...] = acc
        pcar[...] = pltpu.bitcast(pend[-1].astype(BF16), U32)
        return carry

    m_ref[...] = Step(0, 0).set_reference()
    lax.fori_loop(0, NP, attn_body, 0)
    pv_tile((NP - 1) * NC * VR, H - 1, 1, NQ - 1, NC - 1, pltpu.bitcast(pcar[...], BF16), acc_ref[...])

    def exact_attention():
        def exact_step(n, carry):
            pair = n // NQ
            qb = n % NQ
            for par in range(2):
                h = 2 * pair + par

                def score(c, mx):
                    r0 = pl.multiple_of(pair * (S // 2) + c * (CK // 2), CK // 2)
                    kc = pltpu.bitcast(vp0[pl.ds(r0, CK // 2), 0:KD], BF16)
                    w = pltpu.bitcast(qm[h * NQ + qb, 0:KD // 2, :], BF16)
                    s = jnp.dot(kc, w, preferred_element_type=F32)
                    qs[pl.ds(c * 4, 4)] = s.reshape(4, CK // 4, TQ)
                    return jnp.maximum(mx, jnp.max(s.reshape(CK // 8, 8, TQ), axis=0))

                mx = lax.fori_loop(0, NC, score, jnp.full((8, TQ), -jnp.inf, F32))
                mx = jnp.max(mx, axis=0, keepdims=True)

                def weigh(c, acc):
                    p = jnp.exp2(qs[pl.ds(c * 4, 4)].reshape(CK, TQ) - mx).astype(BF16)
                    r0 = pl.multiple_of((pair * NC + c) * VR, 8)
                    return acc + jnp.dot(kbs[1 - par][pl.ds(r0, VR), :], p, preferred_element_type=F32)

                ot[h, :, pl.ds(pl.multiple_of(qb * TQ, TQ), TQ)] = lax.fori_loop(
                    0, NC, weigh, jnp.zeros((VR, TQ), F32))
            return carry

        lax.fori_loop(0, NIT // 2, exact_step, 0)

    cp_wo.wait()

    def cp_o(a):
        rows = pl.ds(a * BLK, BLK)
        return pltpu.make_async_copy(out_v.at[rows], out_hbm.at[rows], osems.at[a])

    def final_body(c, carry):
        dvec = d_ref[...].astype(F32).reshape(1, D)
        gvec = gw_ref[...].astype(F32).reshape(1, D)
        low = lax.broadcasted_iota(jnp.int32, (8, BLK), 0) < 4
        bad = bad_ref[...]

        def inv_dft(b):
            z16 = pl.multiple_of((c * BPC + b) * 16, 16)
            zz = jnp.concatenate([zo[0:NR, lt, pl.ds(z16, 16), :].reshape(NF, 128) for lt in range(LT)], axis=1)
            return jnp.dot(inv_ref[...], zz, preferred_element_type=F32)

        ys = [inv_dft(0)]
        for b in range(BPC):
            rows = pl.ds(pl.multiple_of((c * BPC + b) * BLK, BLK), BLK)
            parts = []
            for j in range(NP):
                if b > 0 and j % 2 == 0:
                    ot[ot_tok, 0:8, 0:128] = ys[b - 1][j * 8:j * 8 + 8, _lanes(j * LT // NP)]
                ae = ot[2 * j, :, rows]
                ao = ot[2 * j + 1, :, rows]
                den = jnp.where(low, ao[0:8], ae[16:24])
                ok = (den >= DEN_LO) & (den <= DEN_HI)
                rec = 1.0 / den
                oe = ae * rec[4:5]
                oo = ao * rec[0:1]
                five = [oe[0:8], oe[8:16], jnp.where(low, oe[16:24], oo[0:8]), oo[8:16], oo[16:24]]
                for piece in five:
                    ok = ok & (jnp.abs(piece) <= OUT_HI)
                bad = jnp.where(ok, bad, 1.0)
                parts += five
            o = jnp.concatenate(parts, axis=0).T
            if b + 1 < BPC:
                ys.append(inv_dft(b + 1))
            att = jnp.dot(o, wo_v[...], preferred_element_type=F32)
            xf = x_v[rows, :].astype(F32)
            gate = jax.nn.sigmoid(jnp.sum(xf * gvec, axis=-1, keepdims=True))
            ssm = xf * (ys[b] + kv[rows, :] * dvec)
            out_v[rows, :] = (gate * att + (1.0 - gate) * ssm).astype(BF16)
            cp_o(c * BPC + b).start()
        bad_ref[...] = bad
        return carry

    def attempt(n, go):
        @pl.when(go > 0)
        def _():
            @pl.when(n > 0)
            def _():
                exact_attention()

            lax.fori_loop(0, NQ, final_body, 0)
            redo_ref[0] = (jnp.max(bad_ref[...]) > 0.0).astype(jnp.int32)
            for a in range(NB):
                cp_o(a).wait()

        return redo_ref[0]

    lax.fori_loop(0, 2, attempt, jnp.int32(1))


@jax.jit
def pallas_gated_mix__mha_block__ssm_conv_h3__prompt_kernel(
    A_x: jax.Array,
    A_wqkv: jax.Array,
    A_wo: jax.Array,
    B_q: jax.Array,
    B_k: jax.Array,
    B_v: jax.Array,
    B_shift_k: jax.Array,
    B_ssm_k: jax.Array,
    B_ssm_D: jax.Array,
    gate_w: jax.Array,
):
    del B_q
    fwd, inv = _dft_consts()
    zeros = jnp.asarray(np.zeros((2,), np.int32))
    hbm = pl.BlockSpec(memory_space=pl.ANY)
    scratch = [
        pltpu.VMEM((NIT, 32, TQ), U32),
        pltpu.VMEM((NIT, 32, TQ), F32),
        pltpu.VMEM((KR + QL * NV + 256, 128), U32),
        pltpu.VMEM((KR + QL * NV + 256, 128), U32),
        pltpu.VMEM((VTR + NV * DH + 256, 128), F32),
        pltpu.VMEM((VTR + NV * DH + 256, 128), F32),
        pltpu.VMEM((NP, NV, 128), F32),
        pltpu.VMEM((NR, LT, 2 * NB * 16, 128), F32),
        pltpu.VMEM((NR + 1, LT, NB * 16, 128), F32),
        pltpu.VMEM((CK // 2, TQ), U32),
        pltpu.VMEM((64, TQ), U32),
        pltpu.VMEM((64, TQ), U32),
        pltpu.VMEM((S, D), F32),
        pltpu.VMEM((NF, D), F32),
        pltpu.VMEM((S, D), BF16),
        pltpu.VMEM((S, D), BF16),
        pltpu.VMEM((NQ, D, TQ), BF16),
        pltpu.VMEM((S, D), BF16),
        pltpu.VMEM((H + 2, VR, S), F32),
        pltpu.VMEM((S + 16, D), BF16),
        pltpu.VMEM((3, D, D), BF16),
        pltpu.VMEM((D, D), BF16),
        pltpu.VMEM((8, TQ), F32),
        pltpu.VMEM((VR, TQ), F32),
        pltpu.VMEM((8, BLK), F32),
        pltpu.VMEM((NF, BLK), BF16),
        pltpu.VMEM((BLK, NF), BF16),
        pltpu.VMEM((KS, D), BF16),
        pltpu.VMEM((D,), BF16),
        pltpu.VMEM((D,), BF16),
        pltpu.SMEM((2,), jnp.int32),
        pltpu.SMEM((1,), jnp.int32),
        pltpu.SemaphoreType.DMA((7, NQ)),
        pltpu.SemaphoreType.DMA((NB,)),
    ]
    out = pl.pallas_call(
        _kernel,
        out_shape=jax.ShapeDtypeStruct((S, D), BF16),
        in_specs=[hbm] * 12,
        out_specs=hbm,
        scratch_shapes=scratch,
        compiler_params=pltpu.CompilerParams(vmem_limit_bytes=124 * 1024 * 1024),
        name="gated_mix_mha_h3",
    )(zeros, A_x.reshape(S, D), A_wqkv, A_wo, B_k.reshape(S, D), B_v.reshape(S, D), B_ssm_k,
      B_shift_k.T, B_ssm_D, gate_w, fwd, inv)
    return out.reshape(1, S, D)
```

```python
import math

import numpy as np
import jax
import jax.numpy as jnp
from jax import lax
import jax.experimental.pallas as pl
import jax.experimental.pallas.tpu as pltpu

S = 2048
D = 640
H = 32
DH = D // H
KS = 4
LT = D // 128

TQ = 512
QL = TQ // 128
CK = 128
NQ = S // TQ
NIT = H * NQ
NC = S // CK
NP = H // 2
UNROLL = 2 * NQ
WL = 2 * DH
KD = 48
VR = 24

GK = 16
GM = CK // GK - 1
NV = NC * GK
KR = NP * (S // 2)
VTR = NP * NC * VR
KB_SETS = 4
KB_PIECES = DH * KB_SETS
KB_SLOTS = 46
REF_SLOT = 4
REF_OFF = 32.0
DEN_LO = 2.0 ** -48
DEN_HI = 2.0 ** 100
OUT_HI = 2.0 ** 126

BLK = 128
NB = S // BLK
NF = 2 * BLK
NR = BLK // 8
BPC = TQ // BLK
KV_ROWS = 32
KV_TILES = 8
MAC_TOK = 2
MAC_SEG = 3

F32 = jnp.float32
BF16 = jnp.bfloat16
U32 = jnp.uint32
NT_DIMS = (((1,), (1,)), ((), ()))

assert NP == NR and BPC * CK == TQ


def _dft_consts():
    f = np.concatenate([np.arange(0, BLK, 2), np.arange(1, BLK, 2)])
    b = np.arange(BLK)
    th = np.pi * (2 * f[:, None] + 1) * b[None, :] / (2 * BLK)
    re = np.cos(th).reshape(NR, 8, BLK)
    im = (-np.sin(th)).reshape(NR, 8, BLK)
    fwd = np.concatenate([re, im], axis=1).reshape(NF, BLK)
    inv = fwd.T / BLK
    return jnp.asarray(fwd, BF16), jnp.asarray(inv, BF16)


def _mm(a, b, dims=(((1,), (0,)), ((), ()))):
    return lax.dot_general(a, b, dims, precision=lax.Precision.DEFAULT, preferred_element_type=F32)


def _kb_pos(slot):
    return min(KB_PIECES, KB_PIECES * max(slot - 1, 0) // KB_SLOTS)


def _lanes(l):
    return slice(l * 128, (l + 1) * 128)


def _kernel(x_hbm, w_hbm, wo_hbm, k_hbm, v_hbm, h_hbm, sk_hbm, d_hbm, gw_hbm,
            fwd_hbm, inv_hbm, out_hbm,
            qm, qs, vp0, vp1, kb0, kb1, kf, uh, zo, pcar,
            kv, hprev, x_v, v_v, h_v, out_v, ot, k_v, w_v, wo_v, wqt, wt0, wt1, m_ref, acc_ref, bad_ref,
            fwd_ref, inv_ref, sk_ref, d_ref, gw_ref, redo_ref, sems, osems):
    vps = (vp0, vp1)
    kbs = (kb0, kb1)
    wts = (wt0, wt1)

    def rows_cp(src, dst, c, sem):
        return pltpu.make_async_copy(src.at[pl.ds(c * TQ, TQ)], dst.at[pl.ds(c * TQ, TQ)], sem)

    def cp_x(c):
        return rows_cp(x_hbm, x_v, c, sems.at[0, c])

    def cp_k(c):
        return rows_cp(k_hbm, k_v, c, sems.at[1, c])

    def cp_v(c):
        return rows_cp(v_hbm, v_v, c, sems.at[2, c])

    def cp_h(c):
        return pltpu.make_async_copy(h_hbm.at[:, pl.ds(c * TQ, TQ)], h_v.at[c], sems.at[3, c])

    def cp_w(n):
        return pltpu.make_async_copy(w_hbm.at[:, pl.ds(n * D, D)], w_v.at[n], sems.at[4, n])

    cp_wo = pltpu.make_async_copy(wo_hbm, wo_v, sems.at[4, 3])
    small = [pltpu.make_async_copy(src, dst, sems.at[5 + n // NQ, n % NQ]) for n, (src, dst) in enumerate(
        [(fwd_hbm, fwd_ref), (sk_hbm, sk_ref), (inv_hbm, inv_ref), (d_hbm, d_ref),
         (gw_hbm, gw_ref)])]
    cp_w(0).start()
    for c in range(NQ):
        cp_x(c).start()
    for cp in small:
        cp.start()
    cp_w(1).start()
    cp_w(2).start()
    for c in range(NQ):
        cp_k(c).start()
        cp_v(c).start()
        cp_h(c).start()
    cp_wo.start()
    hprev[...] = jnp.zeros((NF, D), F32)
    pcar[...] = jnp.zeros((CK // 2, TQ), U32)
    acc_ref[...] = jnp.ones((VR, TQ), F32)
    bad_ref[...] = jnp.zeros((8, BLK), F32)
    cp_w(0).wait()
    wqt[...] = w_v[0].T

    qscale = (DH ** -0.5) * math.log2(math.e)

    def qproj_body(c, carry):
        cp_x(c).wait()
        xc = x_v[pl.ds(pl.multiple_of(c * TQ, TQ), TQ), :]
        qtr = _mm(wqt[...], xc, NT_DIMS) * qscale
        low = lax.broadcasted_iota(jnp.int32, (8, TQ), 0) < 4
        zero8 = jnp.zeros((8, TQ), F32)
        for h in range(H):
            s0 = (h * DH // 8) * 8
            qs[h * NQ + c, 0:VR, :] = qtr[s0:s0 + VR]
            b0 = (h // 2) * WL
            mid = qtr[b0 + 16:b0 + 24]
            if h % 2 == 0:
                wrows = [qtr[b0:b0 + 16], jnp.where(low, mid, 0.0), zero8, zero8, zero8]
            else:
                wrows = [zero8, zero8, jnp.where(low, 0.0, mid), qtr[b0 + 24:b0 + 40], zero8]
            qm[h * NQ + c, 0:KD // 2, :] = pltpu.bitcast(jnp.concatenate(wrows, axis=0).astype(BF16), U32)
        return carry

    lax.fori_loop(0, NQ, qproj_body, 0)

    for cp in small:
        cp.wait()
    cp_w(1).wait()
    cp_w(2).wait()

    def tok_rows(base, idx, n=8):
        return pl.ds(pl.multiple_of(base + jnp.clip(idx, 0, 1) * n, n), n)

    def window(src, j):
        t, off = divmod(j * WL, 128)
        w = src[:, _lanes(t)]
        if off:
            w = pltpu.roll(w, 128 - off, axis=1)
        if off + WL > 128:
            ln = lax.broadcasted_iota(jnp.int32, w.shape, 1)
            w = jnp.where(ln < 128 - off, w, pltpu.roll(src[:, _lanes(t + 1)], 128 - off, axis=1))
        return w

    def proj_body(c, carry):
        r0 = pl.multiple_of(c * TQ, TQ)
        cp_k(c).wait()
        cp_v(c).wait()
        cp_h(c).wait()
        kv_tok = tok_rows(S, c, 16)

        hp = hprev[...].reshape(NR, 16, D)
        for b in range(BPC):
            a16 = pl.multiple_of((c * BPC + b) * 16, 16)
            hraw = _mm(fwd_ref[...], h_v[c, :, b * BLK:(b + 1) * BLK], NT_DIMS).reshape(NR, 16, D)
            e = NR // 2
            hre = jnp.concatenate([hraw[:e, 0:8] - hp[:e, 8:16], hraw[e:, 0:8] + hp[e:, 8:16]], axis=0)
            him = jnp.concatenate([hraw[:e, 8:16] + hp[:e, 0:8], hraw[e:, 8:16] - hp[e:, 0:8]], axis=0)
            for lt in range(LT):
                uh[:, lt, pl.ds(NB * 16 + a16, 8), :] = hre[:, :, _lanes(lt)]
                uh[:, lt, pl.ds(NB * 16 + a16 + 8, 8), :] = him[:, :, _lanes(lt)]
            hp = hraw
        hprev[...] = hp.reshape(NF, D)

        xc = x_v[pl.ds(r0, TQ), :]
        kk = _mm(xc, w_v[1])
        vv = _mm(xc, w_v[2])

        ksel = jnp.concatenate([kk[(b + 1) * CK - GK:(b + 1) * CK] for b in range(BPC)], axis=0)
        kcol = []
        for b in range(BPC):
            kcol.append([jnp.broadcast_to(ksel[b * GK:(b + 1) * GK, d:d + 1], (GK, 128)) for d in range(DH)])
            t0 = pl.multiple_of(VTR + (c * BPC + b) * (GK * DH), GK)
            kb0[pl.ds(t0, DH * GK), :] = jnp.concatenate(kcol[b], axis=0)

        lane = lax.broadcasted_iota(jnp.int32, (TQ // 2, 128), 1)
        ones_l = jnp.where(lane < WL + 2, jnp.uint32(0x3F803F80), jnp.uint32(0))
        r0h = pl.multiple_of(c * (TQ // 2), TQ // 2)
        kkb = pltpu.bitcast(kk.astype(BF16), U32)
        for j in range(NP):
            kw = jnp.where(lane < WL, window(kkb, j), ones_l)
            vp0[pl.ds(j * (S // 2) + r0h, TQ // 2), :] = kw
            vp1[pl.ds(j * (S // 2) + r0h, TQ // 2), :] = kw
            kf[j, pl.ds(pl.multiple_of(c * (BPC * GK), GK), BPC * GK), :] = window(ksel, j)

        for b in range(BPC):
            g0 = pl.multiple_of((c * BPC + b) * GK, GK)
            for l in range(QL):
                sv = None
                for d in range(DH):
                    t = kcol[b][d] * qs[0, d:d + 1, _lanes(l)]
                    sv = t if sv is None else sv + t
                vp0[pl.ds(KR + l * NV + g0, GK), :] = pltpu.bitcast(sv, U32)

        low = lax.broadcasted_iota(jnp.int32, (8, TQ), 0) < 4
        vtr = vv.T
        for j in range(NP):
            b0 = j * WL
            mid = vtr[b0 + 16:b0 + 24]
            slabs = (jnp.concatenate([vtr[b0:b0 + 16], jnp.where(low, mid, 1.0)], axis=0),
                     jnp.concatenate([jnp.where(low, 1.0, mid), vtr[b0 + 24:b0 + 40]], axis=0))
            for par in range(2):
                for b in range(BPC):
                    vr0 = pl.multiple_of((j * NC + c * BPC + b) * VR, 8)
                    kbs[1 - par][pl.ds(vr0, VR), :] = slabs[par][:, b * CK:(b + 1) * CK]

        skf = sk_ref[...].astype(F32)
        npc = (TQ // KV_ROWS) * LT
        per_tile = npc // KV_TILES
        for n in range(npc):
            p, lt = divmod(n, LT)
            ls = _lanes(lt)
            tile, tr = divmod(n, per_tile)
            tr0 = (tr * (TQ // 8) // per_tile) * 8
            src = kk if tile < LT else vv
            k_v[kv_tok, 0:128] = pltpu.bitcast(src[tr0:tr0 + 8, _lanes(tile % LT)], BF16)
            p0 = pl.multiple_of(r0 + p * KV_ROWS, KV_ROWS)
            cur = k_v[pl.ds(p0, KV_ROWS), ls].astype(F32)
            prev = k_v[pl.ds(pl.multiple_of(jnp.maximum(p0 - 16, 0), 16), 16), ls].astype(F32)[8:16]
            if p == 0:
                prev = jnp.where(c > 0, prev, 0.0)
            ext = jnp.concatenate([prev, cur], axis=0)
            ksh = cur * skf[0:1, ls]
            for t in range(1, KS):
                ksh = ksh + ext[8 - t:8 - t + KV_ROWS] * skf[t:t + 1, ls]
            kv[pl.ds(p0, KV_ROWS), ls] = ksh * v_v[pl.ds(p0, KV_ROWS), ls].astype(F32)

        for b in range(BPC):
            a16 = pl.multiple_of((c * BPC + b) * 16, 16)
            ub = kv[pl.ds(pl.multiple_of(r0 + b * BLK, BLK), BLK), :]
            uf = _mm(fwd_ref[...], ub.astype(BF16)).reshape(NR, 16, D)
            for lt in range(LT):
                uh[:, lt, pl.ds(a16, 16), :] = uf[:, :, _lanes(lt)]
        return carry

    lax.fori_loop(0, NQ, proj_body, 0)

    def build_kb(pair, par, piece, kb_tok, tok):
        d, q = divmod(piece, KB_SETS)
        n = NV // KB_SETS
        ln = par * DH + d
        val = jnp.broadcast_to(kf[pair, q * n:(q + 1) * n, ln:ln + 1], (n, 128))
        kbs[par][kb_tok, :] = tok
        for k in range(n // GK):
            g = q * (n // GK) + k
            kbs[par][pl.ds(VTR + (g * DH + d) * GK, GK), :] = val[k * GK:(k + 1) * GK]

    class SpecMac:
        def __init__(self, r):
            self.r = r
            self.items = [(lt, a, j) for lt in range(LT) for a in range(NB) for j in range(a + 1)]
            self.per = -(-len(self.items) // ((UNROLL * NC - 2) * MAC_TOK))
            self.tok = tok_rows(0, r)
            self.pos = 0
            self.zr = None
            self.zi = None

        def run(self, tok):
            r = self.r
            for lt, a, j in self.items[self.pos:self.pos + self.per]:
                hb = (NB + j) * 16
                ub = (a - j) * 16
                hr = uh[r, lt, hb:hb + 8, :]
                hi = uh[r, lt, hb + 8:hb + 16, :]
                ur = uh[r, lt, ub:ub + 8, :]
                ui = uh[r, lt, ub + 8:ub + 16, :]
                tr = hr * ur - hi * ui
                ti = hr * ui + hi * ur
                if j > 0 and j % MAC_SEG == 0:
                    self.zr = zo[r, lt, a * 16:a * 16 + 8, :]
                    self.zi = zo[r, lt, a * 16 + 8:a * 16 + 16, :]
                self.zr = tr if j == 0 else self.zr + tr
                self.zi = ti if j == 0 else self.zi + ti
                if j == a or j % MAC_SEG == MAC_SEG - 1:
                    zo[NR, 0, self.tok, :] = tok
                    zo[r, lt, a * 16:a * 16 + 8, :] = self.zr
                    zo[r, lt, a * 16 + 8:a * 16 + 16, :] = self.zi
            self.pos += self.per

    class Step:
        def __init__(self, u, i):
            self.par = (u // NQ) % 2
            self.buf = vps[u % 2]
            self.wt = wts[u % 2]
            self.i = i
            self.pos = 0

        def vpu_piece(self, vp_tok, tok):
            g, l = self.pos % NC, (self.pos + self.pos // NC) % QL
            self.pos += 1
            sv = [None, None]
            for d in range(DH):
                qr = 4 * self.par + d
                t = kbs[self.par][pl.ds(VTR + (g * DH + d) * GK, GK), :] * qs[self.i, qr:qr + 1, _lanes(l)]
                sv[d % 2] = t if d < 2 else sv[d % 2] + t
            if tok is not None:
                self.buf[vp_tok, :] = pltpu.bitcast(tok, U32)
            self.buf[pl.ds(KR + l * NV + g * GK, GK), :] = pltpu.bitcast(sv[0] + sv[1], U32)

        def vpu_scores(self, groups):
            return jnp.concatenate(
                [pltpu.bitcast(self.buf[pl.ds(KR + l * NV + groups[l] * GK, GK), :], F32) for l in range(QL)],
                axis=1).reshape(GK // 8, 8, TQ)

        def set_reference(self):
            mx = jnp.max(jnp.max(self.vpu_scores(range(QL)), axis=0), axis=0, keepdims=True)
            mb = jnp.broadcast_to((mx + REF_OFF).astype(BF16).astype(F32), (8, TQ))
            sub = lax.broadcasted_iota(jnp.int32, (8, TQ), 0)
            self.wt[...] = jnp.where(sub == WL // 2 - 16, pltpu.bitcast(-mb, U32), qm[self.i, 16:24, :])
            return mb

        def weights(self):
            return pltpu.bitcast(jnp.concatenate([qm[self.i, 0:16, :], self.wt[...]], axis=0), BF16)

    def pv_tile(vrow, head, par, qb, t, p, acc):
        pv = _mm(kbs[1 - par][pl.ds(vrow + t * VR, VR), :], p)
        acc = pv if t == 0 else pv + acc
        if t == NC - 1:
            ot[head, :, qb * TQ:(qb + 1) * TQ] = acc
        return acc

    def attn_body(j, carry):
        i0 = UNROLL * j
        m = m_ref[...]
        acc = acc_ref[...]
        mac = SpecMac(j)
        krow = pl.multiple_of(j * (S // 2), S // 2)
        vrow = pl.multiple_of(j * (NC * VR), NC * VR)
        vrow_prev = pl.multiple_of(jnp.maximum(j - 1, 0) * (NC * VR), NC * VR)
        pair_next = jnp.minimum(j + 1, NP - 1)
        kb_tok = tok_rows(VTR + NV * DH, j)
        vp_tok = tok_rows(KR + QL * NV, j)
        pend = (vrow_prev, jnp.where(j > 0, 2 * j - 1, H), 1, NQ - 1, NC - 1, pltpu.bitcast(pcar[...], BF16))
        sprev = None
        sprev2 = None
        nxt = Step(0, i0)
        for u in range(UNROLL):
            last = u == UNROLL - 1
            head = 2 * j + u // NQ
            cur = nxt
            nxt = Step(u + 1, jnp.minimum(i0 + u + 1, NIT - 1) if last else i0 + u + 1)
            for c in range(NC):
                kbuf = cur.buf if (last and c >= 2) else nxt.buf
                parts = []
                for t in range(QL):
                    p1 = GM * (t + 1) // QL
                    for pp in range(GM * t // QL, p1):
                        key0 = c * CK + GK * (GM - 1 - pp)
                        parts.append(kbuf[pl.ds(krow + key0 // 2, GK // 2), 0:KD])
                    jj, src = (2 * p1 - 4, sprev) if p1 >= 2 else (2 * GM - 1, sprev2)
                    nxt.vpu_piece(vp_tok, None if src is None else src[jj * 8:jj * 8 + 8, 0:128])
                kc = pltpu.bitcast(jnp.concatenate(parts, axis=0), BF16)
                s = _mm(kc, cur.weights())
                pe = jnp.exp2(s)
                acc = pv_tile(*pend, acc)
                tile = [pe[pp * GK:(pp + 1) * GK] for pp in range(GM - 1, -1, -1)]
                tile.append(jnp.exp2(cur.vpu_scores([c] * QL) - m[None]).reshape(GK, TQ))
                pend = (vrow, head, cur.par, u % NQ, c, jnp.concatenate(tile, axis=0))
                if c == REF_SLOT:
                    m_next = nxt.set_reference()
                slot = (u % NQ) * NC + c
                for piece in range(_kb_pos(slot), _kb_pos(slot + 1)):
                    jj = (piece - _kb_pos(slot)) * 6 + 1
                    build_kb(pair_next if cur.par else j, 1 - cur.par, piece, kb_tok, s[jj * 8:jj * 8 + 8, 256:384])
                for t in range(MAC_TOK):
                    jj = t * 2 * GM // MAC_TOK
                    mac.run(s[jj * 8:jj * 8 + 8, 128:256])
                sprev2 = sprev
                sprev = s
            m = m_next
        assert mac.pos >= len(mac.items)
        m_ref[...] = m
        acc_ref[...] = acc
        pcar[...] = pltpu.bitcast(pend[-1].astype(BF16), U32)
        return carry

    m_ref[...] = Step(0, 0).set_reference()
    lax.fori_loop(0, NP, attn_body, 0)
    pv_tile((NP - 1) * NC * VR, H - 1, 1, NQ - 1, NC - 1, pltpu.bitcast(pcar[...], BF16), acc_ref[...])

    def exact_attention():
        def exact_step(n, carry):
            pair = n // NQ
            qb = n % NQ
            for par in range(2):
                h = 2 * pair + par

                def score(c, mx):
                    r0 = pl.multiple_of(pair * (S // 2) + c * (CK // 2), CK // 2)
                    kc = pltpu.bitcast(vp0[pl.ds(r0, CK // 2), 0:KD], BF16)
                    w = pltpu.bitcast(qm[h * NQ + qb, 0:KD // 2, :], BF16)
                    s = _mm(kc, w)
                    qs[pl.ds(c * 4, 4)] = s.reshape(4, CK // 4, TQ)
                    return jnp.maximum(mx, jnp.max(s.reshape(CK // 8, 8, TQ), axis=0))

                mx = lax.fori_loop(0, NC, score, jnp.full((8, TQ), -jnp.inf, F32))
                mx = jnp.max(mx, axis=0, keepdims=True)

                def weigh(c, acc):
                    p = jnp.exp2(qs[pl.ds(c * 4, 4)].reshape(CK, TQ) - mx).astype(BF16)
                    r0 = pl.multiple_of((pair * NC + c) * VR, 8)
                    return acc + _mm(kbs[1 - par][pl.ds(r0, VR), :], p)

                ot[h, :, pl.ds(pl.multiple_of(qb * TQ, TQ), TQ)] = lax.fori_loop(
                    0, NC, weigh, jnp.zeros((VR, TQ), F32))
            return carry

        lax.fori_loop(0, NIT // 2, exact_step, 0)

    cp_wo.wait()

    def cp_o(a):
        rows = pl.ds(a * BLK, BLK)
        return pltpu.make_async_copy(out_v.at[rows], out_hbm.at[rows], osems.at[a])

    def final_body(c, carry):
        dvec = d_ref[...].astype(F32).reshape(1, D)
        gvec = gw_ref[...].astype(F32).reshape(1, D)
        low = lax.broadcasted_iota(jnp.int32, (8, BLK), 0) < 4
        bad = bad_ref[...]
        ot_tok = tok_rows(0, c)

        def inv_dft(b):
            z16 = pl.multiple_of((c * BPC + b) * 16, 16)
            zz = jnp.concatenate([zo[0:NR, lt, pl.ds(z16, 16), :].reshape(NF, 128) for lt in range(LT)], axis=1)
            return _mm(inv_ref[...], zz)

        ys = [inv_dft(0)]
        for b in range(BPC):
            rows = pl.ds(pl.multiple_of((c * BPC + b) * BLK, BLK), BLK)
            parts = []
            for j in range(NP):
                if b > 0 and j % 2 == 0:
                    ot[H + 1, ot_tok, 0:128] = ys[b - 1][j * 8:j * 8 + 8, _lanes(j * LT // NP)]
                ae = ot[2 * j, :, rows]
                ao = ot[2 * j + 1, :, rows]
                den = jnp.where(low, ao[0:8], ae[16:24])
                ok = (den >= DEN_LO) & (den <= DEN_HI)
                rec = 1.0 / den
                oe = ae * rec[4:5]
                oo = ao * rec[0:1]
                five = [oe[0:8], oe[8:16], jnp.where(low, oe[16:24], oo[0:8]), oo[8:16], oo[16:24]]
                for piece in five:
                    ok = ok & (jnp.abs(piece) <= OUT_HI)
                bad = jnp.where(ok, bad, 1.0)
                parts += five
            o = jnp.concatenate(parts, axis=0).T
            if b + 1 < BPC:
                ys.append(inv_dft(b + 1))
            att = _mm(o, wo_v[...])
            xf = x_v[rows, :].astype(F32)
            gate = jax.nn.sigmoid(jnp.sum(xf * gvec, axis=-1, keepdims=True))
            ssm = xf * (ys[b] + kv[rows, :] * dvec)
            out_v[rows, :] = (gate * att + (1.0 - gate) * ssm).astype(BF16)
            cp_o(c * BPC + b).start()
        bad_ref[...] = bad
        return carry

    def attempt(n, go):
        @pl.when(go > 0)
        def _():
            @pl.when(n > 0)
            def _():
                exact_attention()

            lax.fori_loop(0, NQ, final_body, 0)
            redo_ref[0] = (jnp.max(bad_ref[...]) > 0.0).astype(jnp.int32)
            for a in range(NB):
                cp_o(a).wait()

        return redo_ref[0]

    lax.fori_loop(0, 2, attempt, jnp.int32(1))


@jax.jit
def pallas_gated_mix__mha_block__ssm_conv_h3__prompt_kernel(
    A_x: jax.Array,
    A_wqkv: jax.Array,
    A_wo: jax.Array,
    B_q: jax.Array,
    B_k: jax.Array,
    B_v: jax.Array,
    B_shift_k: jax.Array,
    B_ssm_k: jax.Array,
    B_ssm_D: jax.Array,
    gate_w: jax.Array,
):
    del B_q
    fwd, inv = _dft_consts()
    hbm = pl.BlockSpec(memory_space=pl.ANY)
    scratch = [
        pltpu.VMEM((NIT, 32, TQ), U32),
        pltpu.VMEM((NIT, 32, TQ), F32),
        pltpu.VMEM((KR + QL * NV + 256, 128), U32),
        pltpu.VMEM((KR + QL * NV + 256, 128), U32),
        pltpu.VMEM((VTR + NV * DH + 256, 128), F32),
        pltpu.VMEM((VTR + NV * DH + 256, 128), F32),
        pltpu.VMEM((NP, NV, 128), F32),
        pltpu.VMEM((NR, LT, 2 * NB * 16, 128), F32),
        pltpu.VMEM((NR + 1, LT, NB * 16, 128), F32),
        pltpu.VMEM((CK // 2, TQ), U32),
        pltpu.VMEM((S, D), F32),
        pltpu.VMEM((NF, D), F32),
        pltpu.VMEM((S, D), BF16),
        pltpu.VMEM((S, D), BF16),
        pltpu.VMEM((NQ, D, TQ), BF16),
        pltpu.VMEM((S, D), BF16),
        pltpu.VMEM((H + 2, VR, S), F32),
        pltpu.VMEM((S + 32, D), BF16),
        pltpu.VMEM((3, D, D), BF16),
        pltpu.VMEM((D, D), BF16),
        pltpu.VMEM((D, D), BF16),
        pltpu.VMEM((8, TQ), U32),
        pltpu.VMEM((8, TQ), U32),
        pltpu.VMEM((8, TQ), F32),
        pltpu.VMEM((VR, TQ), F32),
        pltpu.VMEM((8, BLK), F32),
        pltpu.VMEM((NF, BLK), BF16),
        pltpu.VMEM((BLK, NF), BF16),
        pltpu.VMEM((KS, D), BF16),
        pltpu.VMEM((D,), BF16),
        pltpu.VMEM((D,), BF16),
        pltpu.SMEM((1,), jnp.int32),
        pltpu.SemaphoreType.DMA((7, NQ)),
        pltpu.SemaphoreType.DMA((NB,)),
    ]
    out = pl.pallas_call(
        _kernel,
        out_shape=jax.ShapeDtypeStruct((S, D), BF16),
        in_specs=[hbm] * 11,
        out_specs=hbm,
        scratch_shapes=scratch,
        compiler_params=pltpu.CompilerParams(vmem_limit_bytes=124 * 1024 * 1024),
        name="gated_mix_mha_h3",
    )(A_x.reshape(S, D), A_wqkv, A_wo, B_k.reshape(S, D), B_v.reshape(S, D), B_ssm_k,
      B_shift_k.T, B_ssm_D, gate_w, fwd, inv)
    return out.reshape(1, S, D)
```

```python
import math

import numpy as np
import jax
import jax.numpy as jnp
from jax import lax
import jax.experimental.pallas as pl
import jax.experimental.pallas.tpu as pltpu

S = 2048
D = 640
H = 32
DH = D // H
KS = 4
LT = D // 128

TQ = 512
QL = TQ // 128
CK = 128
NQ = S // TQ
NIT = H * NQ
NC = S // CK
NP = H // 2
UNROLL = 2 * NQ
WL = 2 * DH
KD = 48
VR = 24

GK = 16
GM = CK // GK - 1
NV = NC * GK
KR = NP * (S // 2)
VTR = NP * NC * VR
KB_SETS = 4
KB_PIECES = DH * KB_SETS
KB_SLOTS = 46
REF_SLOT = 4
REF_OFF = 32.0
DEN_LO = 2.0 ** -48
DEN_HI = 2.0 ** 100
OUT_HI = 2.0 ** 126

BLK = 128
NB = S // BLK
NF = 2 * BLK
NR = BLK // 8
BPC = TQ // BLK
KV_ROWS = 32
KV_TILES = 10
MAC_TOK = 2
MAC_SEG = 3

F32 = jnp.float32
BF16 = jnp.bfloat16
U32 = jnp.uint32
NT_DIMS = (((1,), (1,)), ((), ()))

assert NP == NR and BPC * CK == TQ


def _dft_consts():
    f = np.concatenate([np.arange(0, BLK, 2), np.arange(1, BLK, 2)])
    b = np.arange(BLK)
    th = np.pi * (2 * f[:, None] + 1) * b[None, :] / (2 * BLK)
    re = np.cos(th).reshape(NR, 8, BLK)
    im = (-np.sin(th)).reshape(NR, 8, BLK)
    fwd = np.concatenate([re, im], axis=1).reshape(NF, BLK)
    inv = fwd.T / BLK
    return jnp.asarray(fwd, BF16), jnp.asarray(inv, BF16)


def _mm(a, b, dims=(((1,), (0,)), ((), ()))):
    return lax.dot_general(a, b, dims, precision=lax.Precision.DEFAULT, preferred_element_type=F32)


def _kb_pos(slot):
    return min(KB_PIECES, KB_PIECES * max(slot - 1, 0) // KB_SLOTS)


def _lanes(l):
    return slice(l * 128, (l + 1) * 128)


def _kernel(x_hbm, w_hbm, wo_hbm, k_hbm, v_hbm, h_hbm, sk_hbm, d_hbm, gw_hbm,
            fwd_hbm, inv_hbm, out_hbm,
            qm, qs, vp0, vp1, kb0, kb1, kf, uh, zo, pcar,
            kv, hprev, x_v, v_v, h_v, out_v, ot, k_v, w_v, wo_v, wqt, wt0, wt1, m_ref, acc_ref, bad_ref,
            fwd_ref, inv_ref, sk_ref, d_ref, gw_ref, redo_ref, sems, osems):
    vps = (vp0, vp1)
    kbs = (kb0, kb1)
    wts = (wt0, wt1)

    def rows_cp(src, dst, c, sem):
        return pltpu.make_async_copy(src.at[pl.ds(c * TQ, TQ)], dst.at[pl.ds(c * TQ, TQ)], sem)

    def cp_x(c):
        return rows_cp(x_hbm, x_v, c, sems.at[0, c])

    def cp_k(c):
        return rows_cp(k_hbm, k_v, c, sems.at[1, c])

    def cp_v(c):
        return rows_cp(v_hbm, v_v, c, sems.at[2, c])

    def cp_h(c):
        return pltpu.make_async_copy(h_hbm.at[:, pl.ds(c * TQ, TQ)], h_v.at[c], sems.at[3, c])

    def cp_w(n):
        return pltpu.make_async_copy(w_hbm.at[:, pl.ds(n * D, D)], w_v.at[n], sems.at[4, n])

    cp_wo = pltpu.make_async_copy(wo_hbm, wo_v, sems.at[4, 3])
    small = [pltpu.make_async_copy(src, dst, sems.at[5 + n // NQ, n % NQ]) for n, (src, dst) in enumerate(
        [(fwd_hbm, fwd_ref), (sk_hbm, sk_ref), (inv_hbm, inv_ref), (d_hbm, d_ref),
         (gw_hbm, gw_ref)])]
    cp_w(0).start()
    for c in range(NQ):
        cp_x(c).start()
    for cp in small:
        cp.start()
    cp_w(1).start()
    cp_w(2).start()
    for c in range(NQ):
        cp_k(c).start()
        cp_v(c).start()
        cp_h(c).start()
    cp_wo.start()
    hprev[...] = jnp.zeros((NF, D), F32)
    pcar[...] = jnp.zeros((CK // 2, TQ), U32)
    acc_ref[...] = jnp.ones((VR, TQ), F32)
    bad_ref[...] = jnp.zeros((8, BLK), F32)
    cp_w(0).wait()
    wqt[...] = w_v[0].T

    qscale = (DH ** -0.5) * math.log2(math.e)

    def qproj_body(c, carry):
        cp_x(c).wait()
        xc = x_v[pl.ds(pl.multiple_of(c * TQ, TQ), TQ), :]
        qtr = (_mm(wqt[...], xc, NT_DIMS) * qscale).astype(BF16).astype(F32)
        low = lax.broadcasted_iota(jnp.int32, (8, TQ), 0) < 4
        zero8 = jnp.zeros((8, TQ), F32)
        for h in range(H):
            s0 = (h * DH // 8) * 8
            qs[h * NQ + c, 0:VR, :] = qtr[s0:s0 + VR]
            b0 = (h // 2) * WL
            mid = qtr[b0 + 16:b0 + 24]
            if h % 2 == 0:
                wrows = [qtr[b0:b0 + 16], jnp.where(low, mid, 0.0), zero8, zero8, zero8]
            else:
                wrows = [zero8, zero8, jnp.where(low, 0.0, mid), qtr[b0 + 24:b0 + 40], zero8]
            qm[h * NQ + c, 0:KD // 2, :] = pltpu.bitcast(jnp.concatenate(wrows, axis=0).astype(BF16), U32)
        return carry

    lax.fori_loop(0, NQ, qproj_body, 0)

    for cp in small:
        cp.wait()
    cp_w(1).wait()
    cp_w(2).wait()

    def tok_rows(base, idx, n=8):
        return pl.ds(pl.multiple_of(base + jnp.clip(idx, 0, 1) * n, n), n)

    def window(src, j):
        t, off = divmod(j * WL, 128)
        w = src[:, _lanes(t)]
        if off:
            w = pltpu.roll(w, 128 - off, axis=1)
        if off + WL > 128:
            ln = lax.broadcasted_iota(jnp.int32, w.shape, 1)
            w = jnp.where(ln < 128 - off, w, pltpu.roll(src[:, _lanes(t + 1)], 128 - off, axis=1))
        return w

    def proj_body(c, carry):
        r0 = pl.multiple_of(c * TQ, TQ)
        cp_k(c).wait()
        cp_v(c).wait()
        cp_h(c).wait()
        kv_tok = tok_rows(S, c, 16)

        xc = x_v[pl.ds(r0, TQ), :]
        kk = _mm(xc, w_v[1])
        vv = _mm(xc, w_v[2])

        ksel = jnp.concatenate([kk[(b + 1) * CK - GK:(b + 1) * CK] for b in range(BPC)], axis=0)
        kcol = []
        for b in range(BPC):
            kcol.append([jnp.broadcast_to(ksel[b * GK:(b + 1) * GK, d:d + 1], (GK, 128)) for d in range(DH)])
            t0 = pl.multiple_of(VTR + (c * BPC + b) * (GK * DH), GK)
            kb0[pl.ds(t0, DH * GK), :] = jnp.concatenate(kcol[b], axis=0)

        lane = lax.broadcasted_iota(jnp.int32, (TQ // 2, 128), 1)
        ones_l = jnp.where(lane < WL + 2, jnp.uint32(0x3F803F80), jnp.uint32(0))
        r0h = pl.multiple_of(c * (TQ // 2), TQ // 2)
        kkb = pltpu.bitcast(kk.astype(BF16), U32)
        for j in range(NP):
            kw = jnp.where(lane < WL, window(kkb, j), ones_l)
            vp0[pl.ds(j * (S // 2) + r0h, TQ // 2), :] = kw
            vp1[pl.ds(j * (S // 2) + r0h, TQ // 2), :] = kw
            kf[j, pl.ds(pl.multiple_of(c * (BPC * GK), GK), BPC * GK), :] = window(ksel, j)

        for b in range(BPC):
            g0 = pl.multiple_of((c * BPC + b) * GK, GK)
            for l in range(QL):
                sv = None
                for d in range(DH):
                    t = kcol[b][d] * qs[0, d:d + 1, _lanes(l)]
                    sv = t if sv is None else sv + t
                vp0[pl.ds(KR + l * NV + g0, GK), :] = pltpu.bitcast(sv, U32)

        low = lax.broadcasted_iota(jnp.int32, (8, TQ), 0) < 4
        vtr = vv.T
        for j in range(NP):
            b0 = j * WL
            mid = vtr[b0 + 16:b0 + 24]
            slabs = (jnp.concatenate([vtr[b0:b0 + 16], jnp.where(low, mid, 1.0)], axis=0),
                     jnp.concatenate([jnp.where(low, 1.0, mid), vtr[b0 + 24:b0 + 40]], axis=0))
            for par in range(2):
                for b in range(BPC):
                    vr0 = pl.multiple_of((j * NC + c * BPC + b) * VR, 8)
                    kbs[1 - par][pl.ds(vr0, VR), :] = slabs[par][:, b * CK:(b + 1) * CK]

        skf = sk_ref[...].astype(F32)
        npc = (TQ // KV_ROWS) * LT
        per_tile = npc // KV_TILES
        for n in range(npc):
            p, lt = divmod(n, LT)
            ls = _lanes(lt)
            tile, tr = divmod(n, per_tile)
            tr0 = (tr * (TQ // 8) // per_tile) * 8
            src = kk if tile < LT else vv
            k_v[kv_tok, 0:128] = pltpu.bitcast(src[tr0:tr0 + 8, _lanes(tile % LT)], BF16)
            p0 = pl.multiple_of(r0 + p * KV_ROWS, KV_ROWS)
            cur = k_v[pl.ds(p0, KV_ROWS), ls].astype(F32)
            prev = k_v[pl.ds(pl.multiple_of(jnp.maximum(p0 - 16, 0), 16), 16), ls].astype(F32)[8:16]
            if p == 0:
                prev = jnp.where(c > 0, prev, 0.0)
            ext = jnp.concatenate([prev, cur], axis=0)
            ksh = cur * skf[0:1, ls]
            for t in range(1, KS):
                ksh = ksh + ext[8 - t:8 - t + KV_ROWS] * skf[t:t + 1, ls]
            kv[pl.ds(p0, KV_ROWS), ls] = ksh * v_v[pl.ds(p0, KV_ROWS), ls].astype(F32)

        hp = hprev[...].reshape(NR, 16, D)
        for b in range(BPC):
            a16 = pl.multiple_of((c * BPC + b) * 16, 16)
            hraw = _mm(fwd_ref[...], h_v[c, :, b * BLK:(b + 1) * BLK], NT_DIMS).reshape(NR, 16, D)
            e = NR // 2
            hre = jnp.concatenate([hraw[:e, 0:8] - hp[:e, 8:16], hraw[e:, 0:8] + hp[e:, 8:16]], axis=0)
            him = jnp.concatenate([hraw[:e, 8:16] + hp[:e, 0:8], hraw[e:, 8:16] - hp[e:, 0:8]], axis=0)
            for lt in range(LT):
                uh[:, lt, pl.ds(NB * 16 + a16, 8), :] = hre[:, :, _lanes(lt)]
                uh[:, lt, pl.ds(NB * 16 + a16 + 8, 8), :] = him[:, :, _lanes(lt)]
            hp = hraw
        hprev[...] = hp.reshape(NF, D)

        for b in range(BPC):
            a16 = pl.multiple_of((c * BPC + b) * 16, 16)
            ub = kv[pl.ds(pl.multiple_of(r0 + b * BLK, BLK), BLK), :]
            uf = _mm(fwd_ref[...], ub.astype(BF16)).reshape(NR, 16, D)
            for lt in range(LT):
                uh[:, lt, pl.ds(a16, 16), :] = uf[:, :, _lanes(lt)]
        return carry

    lax.fori_loop(0, NQ, proj_body, 0)

    def build_kb(pair, par, piece, kb_tok, tok):
        d, q = divmod(piece, KB_SETS)
        n = NV // KB_SETS
        ln = par * DH + d
        val = jnp.broadcast_to(kf[pair, q * n:(q + 1) * n, ln:ln + 1], (n, 128))
        kbs[par][kb_tok, :] = tok
        for k in range(n // GK):
            g = q * (n // GK) + k
            kbs[par][pl.ds(VTR + (g * DH + d) * GK, GK), :] = val[k * GK:(k + 1) * GK]

    class SpecMac:
        def __init__(self, r):
            self.r = r
            self.items = [(lt, a, j) for lt in range(LT) for a in range(NB) for j in range(a + 1)]
            self.per = -(-len(self.items) // ((UNROLL * NC - 2) * MAC_TOK))
            self.tok = tok_rows(0, r)
            self.pos = 0
            self.zr = None
            self.zi = None

        def run(self, tok):
            r = self.r
            for lt, a, j in self.items[self.pos:self.pos + self.per]:
                hb = (NB + j) * 16
                ub = (a - j) * 16
                hr = uh[r, lt, hb:hb + 8, :]
                hi = uh[r, lt, hb + 8:hb + 16, :]
                ur = uh[r, lt, ub:ub + 8, :]
                ui = uh[r, lt, ub + 8:ub + 16, :]
                tr = hr * ur - hi * ui
                ti = hr * ui + hi * ur
                if j > 0 and j % MAC_SEG == 0:
                    self.zr = zo[r, lt, a * 16:a * 16 + 8, :]
                    self.zi = zo[r, lt, a * 16 + 8:a * 16 + 16, :]
                self.zr = tr if j == 0 else self.zr + tr
                self.zi = ti if j == 0 else self.zi + ti
                if j == a or j % MAC_SEG == MAC_SEG - 1:
                    zo[NR, 0, self.tok, :] = tok
                    zo[r, lt, a * 16:a * 16 + 8, :] = self.zr
                    zo[r, lt, a * 16 + 8:a * 16 + 16, :] = self.zi
            self.pos += self.per

    class Step:
        def __init__(self, u, i):
            self.par = (u // NQ) % 2
            self.buf = vps[u % 2]
            self.wt = wts[u % 2]
            self.i = i
            self.pos = 0

        def vpu_piece(self, vp_tok, tok):
            g, l = self.pos % NC, (self.pos + self.pos // NC) % QL
            self.pos += 1
            sv = [None, None]
            for d in range(DH):
                qr = 4 * self.par + d
                t = kbs[self.par][pl.ds(VTR + (g * DH + d) * GK, GK), :] * qs[self.i, qr:qr + 1, _lanes(l)]
                sv[d % 2] = t if d < 2 else sv[d % 2] + t
            if tok is not None:
                self.buf[vp_tok, :] = pltpu.bitcast(tok, U32)
            self.buf[pl.ds(KR + l * NV + g * GK, GK), :] = pltpu.bitcast(sv[0] + sv[1], U32)

        def vpu_scores(self, groups):
            return jnp.concatenate(
                [pltpu.bitcast(self.buf[pl.ds(KR + l * NV + groups[l] * GK, GK), :], F32) for l in range(QL)],
                axis=1).reshape(GK // 8, 8, TQ)

        def set_reference(self):
            mx = jnp.max(jnp.max(self.vpu_scores(range(QL)), axis=0), axis=0, keepdims=True)
            bits = pltpu.bitcast(jnp.broadcast_to(-REF_OFF - mx, (8, TQ)), U32) & jnp.uint32(0xFFFF0000)
            sub = lax.broadcasted_iota(jnp.int32, (8, TQ), 0)
            self.wt[...] = jnp.where(sub == WL // 2 - 16, bits, qm[self.i, 16:24, :])
            return pltpu.bitcast(bits, F32)

        def weights(self):
            return pltpu.bitcast(jnp.concatenate([qm[self.i, 0:16, :], self.wt[...]], axis=0), BF16)

    def pv_tile(vrow, head, par, qb, t, p, acc):
        pv = _mm(kbs[1 - par][pl.ds(vrow + t * VR, VR), :], p)
        acc = pv if t == 0 else pv + acc
        if t == NC - 1:
            ot[head, :, qb * TQ:(qb + 1) * TQ] = acc
        return acc

    def attn_body(j, carry):
        i0 = UNROLL * j
        m = m_ref[...]
        acc = acc_ref[...]
        mac = SpecMac(j)
        krow = pl.multiple_of(j * (S // 2), S // 2)
        vrow = pl.multiple_of(j * (NC * VR), NC * VR)
        vrow_prev = pl.multiple_of(jnp.maximum(j - 1, 0) * (NC * VR), NC * VR)
        pair_next = jnp.minimum(j + 1, NP - 1)
        kb_tok = tok_rows(VTR + NV * DH, j)
        vp_tok = tok_rows(KR + QL * NV, j)
        pend = (vrow_prev, jnp.where(j > 0, 2 * j - 1, H), 1, NQ - 1, NC - 1, pltpu.bitcast(pcar[...], BF16))
        sprev = None
        sprev2 = None
        nxt = Step(0, i0)
        for u in range(UNROLL):
            last = u == UNROLL - 1
            head = 2 * j + u // NQ
            cur = nxt
            nxt = Step(u + 1, jnp.minimum(i0 + u + 1, NIT - 1) if last else i0 + u + 1)
            for c in range(NC):
                kbuf = cur.buf if (last and c >= 2) else nxt.buf
                parts = []
                for t in range(QL):
                    p1 = GM * (t + 1) // QL
                    for pp in range(GM * t // QL, p1):
                        key0 = c * CK + GK * (GM - 1 - pp)
                        parts.append(kbuf[pl.ds(krow + key0 // 2, GK // 2), 0:KD])
                    jj, src = (2 * p1 - 4, sprev) if p1 >= 2 else (2 * GM - 1, sprev2)
                    nxt.vpu_piece(vp_tok, None if src is None else src[jj * 8:jj * 8 + 8, 0:128])
                kc = pltpu.bitcast(jnp.concatenate(parts, axis=0), BF16)
                s = _mm(kc, cur.weights())
                pe = jnp.exp2(s)
                acc = pv_tile(*pend, acc)
                tile = [pe[pp * GK:(pp + 1) * GK] for pp in range(GM - 1, -1, -1)]
                tile.append(jnp.exp2(cur.vpu_scores([c] * QL) + m[None]).reshape(GK, TQ))
                pend = (vrow, head, cur.par, u % NQ, c, jnp.concatenate(tile, axis=0))
                if c == REF_SLOT:
                    m_next = nxt.set_reference()
                slot = (u % NQ) * NC + c
                for piece in range(_kb_pos(slot), _kb_pos(slot + 1)):
                    jj = (piece - _kb_pos(slot)) * 6 + 1
                    build_kb(pair_next if cur.par else j, 1 - cur.par, piece, kb_tok, s[jj * 8:jj * 8 + 8, 256:384])
                for t in range(MAC_TOK):
                    jj = t * 2 * GM // MAC_TOK
                    mac.run(s[jj * 8:jj * 8 + 8, 128:256])
                sprev2 = sprev
                sprev = s
            m = m_next
        assert mac.pos >= len(mac.items)
        m_ref[...] = m
        acc_ref[...] = acc
        pcar[...] = pltpu.bitcast(pend[-1].astype(BF16), U32)
        return carry

    m_ref[...] = Step(0, 0).set_reference()
    lax.fori_loop(0, NP, attn_body, 0)
    pv_tile((NP - 1) * NC * VR, H - 1, 1, NQ - 1, NC - 1, pltpu.bitcast(pcar[...], BF16), acc_ref[...])

    def exact_attention():
        def exact_step(n, carry):
            pair = n // NQ
            qb = n % NQ
            for par in range(2):
                h = 2 * pair + par

                def score(c, mx):
                    r0 = pl.multiple_of(pair * (S // 2) + c * (CK // 2), CK // 2)
                    kc = pltpu.bitcast(vp0[pl.ds(r0, CK // 2), 0:KD], BF16)
                    w = pltpu.bitcast(qm[h * NQ + qb, 0:KD // 2, :], BF16)
                    s = _mm(kc, w)
                    qs[pl.ds(c * 4, 4)] = s.reshape(4, CK // 4, TQ)
                    return jnp.maximum(mx, jnp.max(s.reshape(CK // 8, 8, TQ), axis=0))

                mx = lax.fori_loop(0, NC, score, jnp.full((8, TQ), -jnp.inf, F32))
                mx = jnp.max(mx, axis=0, keepdims=True)

                def weigh(c, acc):
                    p = jnp.exp2(qs[pl.ds(c * 4, 4)].reshape(CK, TQ) - mx).astype(BF16)
                    r0 = pl.multiple_of((pair * NC + c) * VR, 8)
                    return acc + _mm(kbs[1 - par][pl.ds(r0, VR), :], p)

                ot[h, :, pl.ds(pl.multiple_of(qb * TQ, TQ), TQ)] = lax.fori_loop(
                    0, NC, weigh, jnp.zeros((VR, TQ), F32))
            return carry

        lax.fori_loop(0, NIT // 2, exact_step, 0)

    cp_wo.wait()

    def cp_o(a):
        rows = pl.ds(a * BLK, BLK)
        return pltpu.make_async_copy(out_v.at[rows], out_hbm.at[rows], osems.at[a])

    def final_body(c, carry):
        dvec = d_ref[...].astype(F32).reshape(1, D)
        gvec = gw_ref[...].astype(F32).reshape(1, D)
        low = lax.broadcasted_iota(jnp.int32, (8, BLK), 0) < 4
        bad = bad_ref[...]
        ot_tok = tok_rows(0, c)

        def inv_dft(b):
            z16 = pl.multiple_of((c * BPC + b) * 16, 16)
            zz = jnp.concatenate([zo[0:NR, lt, pl.ds(z16, 16), :].reshape(NF, 128) for lt in range(LT)], axis=1)
            return _mm(inv_ref[...], zz)

        ys = [inv_dft(0)]
        for b in range(BPC):
            rows = pl.ds(pl.multiple_of((c * BPC + b) * BLK, BLK), BLK)
            parts = []
            for j in range(NP):
                if b > 0 and j % 2 == 0:
                    ot[H + 1, ot_tok, 0:128] = ys[b - 1][j * 8:j * 8 + 8, _lanes(j * LT // NP)]
                ae = ot[2 * j, :, rows]
                ao = ot[2 * j + 1, :, rows]
                den = jnp.where(low, ao[0:8], ae[16:24])
                ok = (den >= DEN_LO) & (den <= DEN_HI)
                rec = 1.0 / den
                oe = ae * rec[4:5]
                oo = ao * rec[0:1]
                five = [oe[0:8], oe[8:16], jnp.where(low, oe[16:24], oo[0:8]), oo[8:16], oo[16:24]]
                for piece in five:
                    ok = ok & (jnp.abs(piece) <= OUT_HI)
                bad = jnp.where(ok, bad, 1.0)
                parts += five
            o = jnp.concatenate(parts, axis=0).T
            if b + 1 < BPC:
                ys.append(inv_dft(b + 1))
            att = _mm(o, wo_v[...])
            xf = x_v[rows, :].astype(F32)
            gate = jax.nn.sigmoid(jnp.sum(xf * gvec, axis=-1, keepdims=True))
            ssm = xf * (ys[b] + kv[rows, :] * dvec)
            out_v[rows, :] = (gate * att + (1.0 - gate) * ssm).astype(BF16)
            cp_o(c * BPC + b).start()
        bad_ref[...] = bad
        return carry

    def attempt(n, go):
        @pl.when(go > 0)
        def _():
            @pl.when(n > 0)
            def _():
                exact_attention()

            lax.fori_loop(0, NQ, final_body, 0)
            redo_ref[0] = (jnp.max(bad_ref[...]) > 0.0).astype(jnp.int32)
            for a in range(NB):
                cp_o(a).wait()

        return redo_ref[0]

    lax.fori_loop(0, 2, attempt, jnp.int32(1))


@jax.jit
def pallas_gated_mix__mha_block__ssm_conv_h3__prompt_kernel(
    A_x: jax.Array,
    A_wqkv: jax.Array,
    A_wo: jax.Array,
    B_q: jax.Array,
    B_k: jax.Array,
    B_v: jax.Array,
    B_shift_k: jax.Array,
    B_ssm_k: jax.Array,
    B_ssm_D: jax.Array,
    gate_w: jax.Array,
):
    del B_q
    fwd, inv = _dft_consts()
    hbm = pl.BlockSpec(memory_space=pl.ANY)
    scratch = [
        pltpu.VMEM((NIT, 32, TQ), U32),
        pltpu.VMEM((NIT, 32, TQ), F32),
        pltpu.VMEM((KR + QL * NV + 256, 128), U32),
        pltpu.VMEM((KR + QL * NV + 256, 128), U32),
        pltpu.VMEM((VTR + NV * DH + 256, 128), F32),
        pltpu.VMEM((VTR + NV * DH + 256, 128), F32),
        pltpu.VMEM((NP, NV, 128), F32),
        pltpu.VMEM((NR, LT, 2 * NB * 16, 128), F32),
        pltpu.VMEM((NR + 1, LT, NB * 16, 128), F32),
        pltpu.VMEM((CK // 2, TQ), U32),
        pltpu.VMEM((S, D), F32),
        pltpu.VMEM((NF, D), F32),
        pltpu.VMEM((S, D), BF16),
        pltpu.VMEM((S, D), BF16),
        pltpu.VMEM((NQ, D, TQ), BF16),
        pltpu.VMEM((S, D), BF16),
        pltpu.VMEM((H + 2, VR, S), F32),
        pltpu.VMEM((S + 32, D), BF16),
        pltpu.VMEM((3, D, D), BF16),
        pltpu.VMEM((D, D), BF16),
        pltpu.VMEM((D, D), BF16),
        pltpu.VMEM((8, TQ), U32),
        pltpu.VMEM((8, TQ), U32),
        pltpu.VMEM((8, TQ), F32),
        pltpu.VMEM((VR, TQ), F32),
        pltpu.VMEM((8, BLK), F32),
        pltpu.VMEM((NF, BLK), BF16),
        pltpu.VMEM((BLK, NF), BF16),
        pltpu.VMEM((KS, D), BF16),
        pltpu.VMEM((D,), BF16),
        pltpu.VMEM((D,), BF16),
        pltpu.SMEM((1,), jnp.int32),
        pltpu.SemaphoreType.DMA((7, NQ)),
        pltpu.SemaphoreType.DMA((NB,)),
    ]
    out = pl.pallas_call(
        _kernel,
        out_shape=jax.ShapeDtypeStruct((S, D), BF16),
        in_specs=[hbm] * 11,
        out_specs=hbm,
        scratch_shapes=scratch,
        compiler_params=pltpu.CompilerParams(vmem_limit_bytes=124 * 1024 * 1024),
        name="gated_mix_mha_h3",
    )(A_x.reshape(S, D), A_wqkv, A_wo, B_k.reshape(S, D), B_v.reshape(S, D), B_ssm_k,
      B_shift_k.T, B_ssm_D, gate_w, fwd, inv)
    return out.reshape(1, S, D)
```

```python
import math

import numpy as np
import jax
import jax.numpy as jnp
from jax import lax
import jax.experimental.pallas as pl
import jax.experimental.pallas.tpu as pltpu

S = 2048
D = 640
H = 32
DH = D // H
KS = 4
LT = D // 128

TQ = 512
QL = TQ // 128
CK = 128
NQ = S // TQ
NIT = H * NQ
NC = S // CK
NP = H // 2
UNROLL = 2 * NQ
WL = 2 * DH
KD = 48
VR = 24

GK = 16
GT = CK // GK
VG = [2 if t in (4, 12) else 1 for t in range(NC)]
VGL = [2, 1, 1, 1] * NQ
GPC = sum(VGL) // NQ
NV = sum(VGL) * GK
VPOS = [sum(VGL[:t + 1]) - VG[t] for t in range(NC)]
ACT = [VPOS[t] + k for t in range(NC) for k in range(VG[t])]
NA = len(ACT)
GKEY = [t * CK + GK * (GT - VG[t] - 1 - p) for t in range(NC) for p in range(GT - VG[t])]
CONS = [GT * t - sum(VG[:t]) for t in range(NC + 1)]
FEED = [0] + [CONS[c] + GT - 1 for c in range(NC)]
KR = NP * (S // 2)
VTR = NP * NC * VR
KB_SETS = 4
KB_PIECES = DH * KB_SETS
KB_SLOTS = 46
REF_SLOT = 4
REF_OFF = 32.0
DEN_LO = 2.0 ** -48
DEN_HI = 2.0 ** 100
OUT_HI = 2.0 ** 126

BLK = 128
NB = S // BLK
NF = 2 * BLK
NR = BLK // 8
BPC = TQ // BLK
KV_ROWS = 32
KV_TILES = 10
MAC_TOK = 3
MAC_SEG = 2

F32 = jnp.float32
BF16 = jnp.bfloat16
U32 = jnp.uint32
NT_DIMS = (((1,), (1,)), ((), ()))

assert NP == NR and BPC * CK == TQ and FEED[NC] == CONS[NC] == len(GKEY)


def _dft_consts():
    f = np.concatenate([np.arange(0, BLK, 2), np.arange(1, BLK, 2)])
    b = np.arange(BLK)
    th = np.pi * (2 * f[:, None] + 1) * b[None, :] / (2 * BLK)
    re = np.cos(th).reshape(NR, 8, BLK)
    im = (-np.sin(th)).reshape(NR, 8, BLK)
    fwd = np.concatenate([re, im], axis=1).reshape(NF, BLK)
    inv = fwd.T / BLK
    return jnp.asarray(fwd, BF16), jnp.asarray(inv, BF16)


def _mm(a, b, dims=(((1,), (0,)), ((), ()))):
    return lax.dot_general(a, b, dims, precision=lax.Precision.DEFAULT, preferred_element_type=F32)


def _kb_pos(slot):
    return min(KB_PIECES, KB_PIECES * max(slot - 1, 0) // KB_SLOTS)


def _lanes(l):
    return slice(l * 128, (l + 1) * 128)


def _kernel(x_hbm, w_hbm, wo_hbm, k_hbm, v_hbm, h_hbm, sk_hbm, d_hbm, gw_hbm,
            fwd_hbm, inv_hbm, out_hbm,
            qm, qs, vp0, vp1, kb0, kb1, kf, uh, zo, pcar,
            kv, hprev, x_v, v_v, h_v, out_v, ot, k_v, w_v, wo_v, wqt, wt0, wt1, m_ref, acc_ref, bad_ref,
            fwd_ref, inv_ref, sk_ref, d_ref, gw_ref, redo_ref, sems, osems):
    vps = (vp0, vp1)
    kbs = (kb0, kb1)
    wts = (wt0, wt1)

    def rows_cp(src, dst, c, sem):
        return pltpu.make_async_copy(src.at[pl.ds(c * TQ, TQ)], dst.at[pl.ds(c * TQ, TQ)], sem)

    def cp_x(c):
        return rows_cp(x_hbm, x_v, c, sems.at[0, c])

    def cp_k(c):
        return rows_cp(k_hbm, k_v, c, sems.at[1, c])

    def cp_v(c):
        return rows_cp(v_hbm, v_v, c, sems.at[2, c])

    def cp_h(c):
        return pltpu.make_async_copy(h_hbm.at[:, pl.ds(c * TQ, TQ)], h_v.at[c], sems.at[3, c])

    def cp_w(n):
        return pltpu.make_async_copy(w_hbm.at[:, pl.ds(n * D, D)], w_v.at[n], sems.at[4, n])

    cp_wo = pltpu.make_async_copy(wo_hbm, wo_v, sems.at[4, 3])
    small = [pltpu.make_async_copy(src, dst, sems.at[5 + n // NQ, n % NQ]) for n, (src, dst) in enumerate(
        [(fwd_hbm, fwd_ref), (sk_hbm, sk_ref), (inv_hbm, inv_ref), (d_hbm, d_ref),
         (gw_hbm, gw_ref)])]
    cp_w(0).start()
    for c in range(NQ):
        cp_x(c).start()
    for cp in small:
        cp.start()
    cp_w(1).start()
    cp_w(2).start()
    for c in range(NQ):
        cp_k(c).start()
        cp_v(c).start()
        cp_h(c).start()
    cp_wo.start()
    hprev[...] = jnp.zeros((NF, D), F32)
    pcar[...] = jnp.zeros((CK // 2, TQ), U32)
    acc_ref[...] = jnp.ones((VR, TQ), F32)
    bad_ref[...] = jnp.zeros((8, BLK), F32)
    cp_w(0).wait()
    wqt[...] = w_v[0].T

    qscale = (DH ** -0.5) * math.log2(math.e)

    def qproj_body(c, carry):
        cp_x(c).wait()
        xc = x_v[pl.ds(pl.multiple_of(c * TQ, TQ), TQ), :]
        qtr = (_mm(wqt[...], xc, NT_DIMS) * qscale).astype(BF16).astype(F32)
        low = lax.broadcasted_iota(jnp.int32, (8, TQ), 0) < 4
        zero8 = jnp.zeros((8, TQ), F32)
        for h in range(H):
            s0 = (h * DH // 8) * 8
            qs[h * NQ + c, 0:VR, :] = qtr[s0:s0 + VR]
            b0 = (h // 2) * WL
            mid = qtr[b0 + 16:b0 + 24]
            if h % 2 == 0:
                wrows = [qtr[b0:b0 + 16], jnp.where(low, mid, 0.0), zero8, zero8, zero8]
            else:
                wrows = [zero8, zero8, jnp.where(low, 0.0, mid), qtr[b0 + 24:b0 + 40], zero8]
            qm[h * NQ + c, 0:KD // 2, :] = pltpu.bitcast(jnp.concatenate(wrows, axis=0).astype(BF16), U32)
        return carry

    lax.fori_loop(0, NQ, qproj_body, 0)

    for cp in small:
        cp.wait()
    cp_w(1).wait()
    cp_w(2).wait()

    def tok_rows(base, idx, n=8):
        return pl.ds(pl.multiple_of(base + jnp.clip(idx, 0, 1) * n, n), n)

    def window(src, j):
        t, off = divmod(j * WL, 128)
        w = src[:, _lanes(t)]
        if off:
            w = pltpu.roll(w, 128 - off, axis=1)
        if off + WL > 128:
            ln = lax.broadcasted_iota(jnp.int32, w.shape, 1)
            w = jnp.where(ln < 128 - off, w, pltpu.roll(src[:, _lanes(t + 1)], 128 - off, axis=1))
        return w

    def proj_body(c, carry):
        r0 = pl.multiple_of(c * TQ, TQ)
        cp_k(c).wait()
        cp_v(c).wait()
        cp_h(c).wait()
        kv_tok = tok_rows(S, c, 16)

        xc = x_v[pl.ds(r0, TQ), :]
        kk = _mm(xc, w_v[1])
        vv = _mm(xc, w_v[2])

        ksel = jnp.concatenate([kk[(b + 1) * CK - GK * VGL[b]:(b + 1) * CK] for b in range(BPC)], axis=0)
        kcol = []
        for b in range(GPC):
            kcol.append([jnp.broadcast_to(ksel[b * GK:(b + 1) * GK, d:d + 1], (GK, 128)) for d in range(DH)])
            t0 = pl.multiple_of(VTR + (c * GPC + b) * (GK * DH), GK)
            kb0[pl.ds(t0, DH * GK), :] = jnp.concatenate(kcol[b], axis=0)

        lane = lax.broadcasted_iota(jnp.int32, (TQ // 2, 128), 1)
        ones_l = jnp.where(lane < WL + 2, jnp.uint32(0x3F803F80), jnp.uint32(0))
        r0h = pl.multiple_of(c * (TQ // 2), TQ // 2)
        kkb = pltpu.bitcast(kk.astype(BF16), U32)
        for j in range(NP):
            kw = jnp.where(lane < WL, window(kkb, j), ones_l)
            vp0[pl.ds(j * (S // 2) + r0h, TQ // 2), :] = kw
            vp1[pl.ds(j * (S // 2) + r0h, TQ // 2), :] = kw
            kf[j, pl.ds(pl.multiple_of(c * (GPC * GK), GK), GPC * GK), :] = window(ksel, j)

        for b in range(GPC):
            g0 = pl.multiple_of((c * GPC + b) * GK, GK)
            for l in range(QL):
                sv = None
                for d in range(DH):
                    t = kcol[b][d] * qs[0, d:d + 1, _lanes(l)]
                    sv = t if sv is None else sv + t
                vp0[pl.ds(KR + l * NV + g0, GK), :] = pltpu.bitcast(sv, U32)

        low = lax.broadcasted_iota(jnp.int32, (8, TQ), 0) < 4
        vtr = vv.T
        for j in range(NP):
            b0 = j * WL
            mid = vtr[b0 + 16:b0 + 24]
            slabs = (jnp.concatenate([vtr[b0:b0 + 16], jnp.where(low, mid, 1.0)], axis=0),
                     jnp.concatenate([jnp.where(low, 1.0, mid), vtr[b0 + 24:b0 + 40]], axis=0))
            for par in range(2):
                for b in range(BPC):
                    vr0 = pl.multiple_of((j * NC + c * BPC + b) * VR, 8)
                    kbs[1 - par][pl.ds(vr0, VR), :] = slabs[par][:, b * CK:(b + 1) * CK]

        skf = sk_ref[...].astype(F32)
        npc = (TQ // KV_ROWS) * LT
        per_tile = npc // KV_TILES
        for n in range(npc):
            p, lt = divmod(n, LT)
            ls = _lanes(lt)
            tile, tr = divmod(n, per_tile)
            tr0 = (tr * (TQ // 8) // per_tile) * 8
            src = kk if tile < LT else vv
            k_v[kv_tok, 0:128] = pltpu.bitcast(src[tr0:tr0 + 8, _lanes(tile % LT)], BF16)
            p0 = pl.multiple_of(r0 + p * KV_ROWS, KV_ROWS)
            cur = k_v[pl.ds(p0, KV_ROWS), ls].astype(F32)
            prev = k_v[pl.ds(pl.multiple_of(jnp.maximum(p0 - 16, 0), 16), 16), ls].astype(F32)[8:16]
            if p == 0:
                prev = jnp.where(c > 0, prev, 0.0)
            ext = jnp.concatenate([prev, cur], axis=0)
            ksh = cur * skf[0:1, ls]
            for t in range(1, KS):
                ksh = ksh + ext[8 - t:8 - t + KV_ROWS] * skf[t:t + 1, ls]
            kv[pl.ds(p0, KV_ROWS), ls] = ksh * v_v[pl.ds(p0, KV_ROWS), ls].astype(F32)

        hp = hprev[...].reshape(NR, 16, D)
        for b in range(BPC):
            a16 = pl.multiple_of((c * BPC + b) * 16, 16)
            hraw = _mm(fwd_ref[...], h_v[c, :, b * BLK:(b + 1) * BLK], NT_DIMS).reshape(NR, 16, D)
            e = NR // 2
            hre = jnp.concatenate([hraw[:e, 0:8] - hp[:e, 8:16], hraw[e:, 0:8] + hp[e:, 8:16]], axis=0)
            him = jnp.concatenate([hraw[:e, 8:16] + hp[:e, 0:8], hraw[e:, 8:16] - hp[e:, 0:8]], axis=0)
            for lt in range(LT):
                uh[:, lt, pl.ds(NB * 16 + a16, 8), :] = hre[:, :, _lanes(lt)]
                uh[:, lt, pl.ds(NB * 16 + a16 + 8, 8), :] = him[:, :, _lanes(lt)]
            hp = hraw
        hprev[...] = hp.reshape(NF, D)

        for b in range(BPC):
            a16 = pl.multiple_of((c * BPC + b) * 16, 16)
            ub = kv[pl.ds(pl.multiple_of(r0 + b * BLK, BLK), BLK), :]
            uf = _mm(fwd_ref[...], ub.astype(BF16)).reshape(NR, 16, D)
            for lt in range(LT):
                uh[:, lt, pl.ds(a16, 16), :] = uf[:, :, _lanes(lt)]
        return carry

    lax.fori_loop(0, NQ, proj_body, 0)

    def build_kb(pair, par, piece, kb_tok, tok):
        d, q = divmod(piece, KB_SETS)
        ln = par * DH + d
        gs = ACT[NA * q // KB_SETS:NA * (q + 1) // KB_SETS]
        vals = [jnp.broadcast_to(kf[pair, g * GK:(g + 1) * GK, ln:ln + 1], (GK, 128)) for g in gs]
        kbs[par][kb_tok, :] = tok
        for g, val in zip(gs, vals):
            kbs[par][pl.ds(VTR + (g * DH + d) * GK, GK), :] = val

    class SpecMac:
        def __init__(self, r):
            self.r = r
            self.items = [(lt, a, j) for lt in range(LT) for a in range(NB) for j in range(a + 1)]
            self.per = -(-len(self.items) // ((UNROLL * NC - 2) * MAC_TOK))
            self.tok = tok_rows(0, r)
            self.pos = 0
            self.zr = None
            self.zi = None

        def run(self, tok):
            r = self.r
            for lt, a, j in self.items[self.pos:self.pos + self.per]:
                hb = (NB + j) * 16
                ub = (a - j) * 16
                hr = uh[r, lt, hb:hb + 8, :]
                hi = uh[r, lt, hb + 8:hb + 16, :]
                ur = uh[r, lt, ub:ub + 8, :]
                ui = uh[r, lt, ub + 8:ub + 16, :]
                tr = hr * ur - hi * ui
                ti = hr * ui + hi * ur
                if j > 0 and j % MAC_SEG == 0:
                    self.zr = zo[r, lt, a * 16:a * 16 + 8, :]
                    self.zi = zo[r, lt, a * 16 + 8:a * 16 + 16, :]
                self.zr = tr if j == 0 else self.zr + tr
                self.zi = ti if j == 0 else self.zi + ti
                if j == a or j % MAC_SEG == MAC_SEG - 1:
                    zo[NR, 0, self.tok, :] = tok
                    zo[r, lt, a * 16:a * 16 + 8, :] = self.zr
                    zo[r, lt, a * 16 + 8:a * 16 + 16, :] = self.zi
            self.pos += self.per

    class Step:
        def __init__(self, u, i):
            self.par = (u // NQ) % 2
            self.buf = vps[u % 2]
            self.wt = wts[u % 2]
            self.i = i
            self.pos = 0

        def vpu_piece(self, vp_tok, tok):
            r, k = divmod(self.pos, NA)
            g, l = ACT[k], (k + r) % QL
            self.pos += 1
            sv = [None, None]
            for d in range(DH):
                qr = 4 * self.par + d
                t = kbs[self.par][pl.ds(VTR + (g * DH + d) * GK, GK), :] * qs[self.i, qr:qr + 1, _lanes(l)]
                sv[d % 2] = t if d < 2 else sv[d % 2] + t
            if tok is not None:
                self.buf[vp_tok, :] = pltpu.bitcast(tok, U32)
            self.buf[pl.ds(KR + l * NV + g * GK, GK), :] = pltpu.bitcast(sv[0] + sv[1], U32)

        def vpu_scores(self, groups, n=1):
            return jnp.concatenate(
                [pltpu.bitcast(self.buf[pl.ds(KR + l * NV + groups[l] * GK, n * GK), :], F32) for l in range(QL)],
                axis=1).reshape(n * GK // 8, 8, TQ)

        def set_reference(self):
            mx = jnp.max(jnp.max(self.vpu_scores(ACT[:QL]), axis=0), axis=0, keepdims=True)
            bits = pltpu.bitcast(jnp.broadcast_to(-REF_OFF - mx, (8, TQ)), U32) & jnp.uint32(0xFFFF0000)
            sub = lax.broadcasted_iota(jnp.int32, (8, TQ), 0)
            self.wt[...] = jnp.where(sub == WL // 2 - 16, bits, qm[self.i, 16:24, :])
            return pltpu.bitcast(bits, F32)

        def weights(self):
            return pltpu.bitcast(jnp.concatenate([qm[self.i, 0:16, :], self.wt[...]], axis=0), BF16)

    def pv_tile(vrow, head, par, qb, t, p, acc):
        pv = _mm(kbs[1 - par][pl.ds(vrow + t * VR, VR), :], p)
        acc = pv if t == 0 else pv + acc
        if t == NC - 1:
            ot[head, :, qb * TQ:(qb + 1) * TQ] = acc
        return acc

    def attn_body(j, carry):
        i0 = UNROLL * j
        m = m_ref[...]
        acc = acc_ref[...]
        mac = SpecMac(j)
        krow = pl.multiple_of(j * (S // 2), S // 2)
        vrow = pl.multiple_of(j * (NC * VR), NC * VR)
        vrow_prev = pl.multiple_of(jnp.maximum(j - 1, 0) * (NC * VR), NC * VR)
        pair_next = jnp.minimum(j + 1, NP - 1)
        kb_tok = tok_rows(VTR + NV * DH, j)
        vp_tok = tok_rows(KR + QL * NV, j)
        pend = (vrow_prev, jnp.where(j > 0, 2 * j - 1, H), 1, NQ - 1, NC - 1, pltpu.bitcast(pcar[...], BF16))
        sprev = None
        sprev2 = None
        nxt = Step(0, i0)
        for u in range(UNROLL):
            last = u == UNROLL - 1
            head = 2 * j + u // NQ
            cur = nxt
            nxt = Step(u + 1, jnp.minimum(i0 + u + 1, NIT - 1) if last else i0 + u + 1)
            groups = {}
            for c in range(NC):
                kbuf = cur.buf if (last and c >= 2) else nxt.buf
                parts = []
                n0, npar = FEED[c], FEED[c + 1] - FEED[c]
                at = QL * NA * (c + 1) // NC - QL * NA * c // NC
                for t in range(at):
                    p1 = npar * (t + 1) // at
                    for pp in range(npar * t // at, p1):
                        parts.append(kbuf[pl.ds(krow + GKEY[n0 + pp] // 2, GK // 2), 0:KD])
                    src = sprev if p1 >= 2 else sprev2
                    tok = None
                    if src is not None:
                        jj = src.shape[0] // 8 - 1
                        jj = min(2 * p1 - 4, jj) if p1 >= 2 else jj
                        tok = src[jj * 8:jj * 8 + 8, 0:128]
                    nxt.vpu_piece(vp_tok, tok)
                kc = pltpu.bitcast(jnp.concatenate(parts, axis=0), BF16)
                s = _mm(kc, cur.weights())
                pe = jnp.exp2(s)
                for pp in range(npar):
                    groups[n0 + pp] = pe[pp * GK:(pp + 1) * GK]
                acc = pv_tile(*pend, acc)
                tile = [groups[n] for n in range(CONS[c + 1] - 1, CONS[c] - 1, -1)]
                tile.append(jnp.exp2(cur.vpu_scores([VPOS[c]] * QL, VG[c]) + m[None]).reshape(VG[c] * GK, TQ))
                pend = (vrow, head, cur.par, u % NQ, c, jnp.concatenate(tile, axis=0))
                if c == REF_SLOT:
                    m_next = nxt.set_reference()
                slot = (u % NQ) * NC + c
                for piece in range(_kb_pos(slot), _kb_pos(slot + 1)):
                    jj = (piece - _kb_pos(slot)) * 6 + 1
                    build_kb(pair_next if cur.par else j, 1 - cur.par, piece, kb_tok, s[jj * 8:jj * 8 + 8, 256:384])
                for t in range(MAC_TOK):
                    jj = t * 2 * npar // MAC_TOK
                    mac.run(s[jj * 8:jj * 8 + 8, 128:256])
                sprev2 = sprev
                sprev = s
            m = m_next
        assert mac.pos >= len(mac.items)
        m_ref[...] = m
        acc_ref[...] = acc
        pcar[...] = pltpu.bitcast(pend[-1].astype(BF16), U32)
        return carry

    m_ref[...] = Step(0, 0).set_reference()
    lax.fori_loop(0, NP, attn_body, 0)
    pv_tile((NP - 1) * NC * VR, H - 1, 1, NQ - 1, NC - 1, pltpu.bitcast(pcar[...], BF16), acc_ref[...])

    def exact_attention():
        def exact_step(n, carry):
            pair = n // NQ
            qb = n % NQ
            for par in range(2):
                h = 2 * pair + par

                def score(c, mx):
                    r0 = pl.multiple_of(pair * (S // 2) + c * (CK // 2), CK // 2)
                    kc = pltpu.bitcast(vp0[pl.ds(r0, CK // 2), 0:KD], BF16)
                    w = pltpu.bitcast(qm[h * NQ + qb, 0:KD // 2, :], BF16)
                    s = _mm(kc, w)
                    qs[pl.ds(c * 4, 4)] = s.reshape(4, CK // 4, TQ)
                    return jnp.maximum(mx, jnp.max(s.reshape(CK // 8, 8, TQ), axis=0))

                mx = lax.fori_loop(0, NC, score, jnp.full((8, TQ), -jnp.inf, F32))
                mx = jnp.max(mx, axis=0, keepdims=True)

                def weigh(c, acc):
                    p = jnp.exp2(qs[pl.ds(c * 4, 4)].reshape(CK, TQ) - mx).astype(BF16)
                    r0 = pl.multiple_of((pair * NC + c) * VR, 8)
                    return acc + _mm(kbs[1 - par][pl.ds(r0, VR), :], p)

                ot[h, :, pl.ds(pl.multiple_of(qb * TQ, TQ), TQ)] = lax.fori_loop(
                    0, NC, weigh, jnp.zeros((VR, TQ), F32))
            return carry

        lax.fori_loop(0, NIT // 2, exact_step, 0)

    cp_wo.wait()

    def cp_o(a):
        rows = pl.ds(a * BLK, BLK)
        return pltpu.make_async_copy(out_v.at[rows], out_hbm.at[rows], osems.at[a])

    def final_body(c, carry):
        dvec = d_ref[...].astype(F32).reshape(1, D)
        gvec = gw_ref[...].astype(F32).reshape(1, D)
        low = lax.broadcasted_iota(jnp.int32, (8, BLK), 0) < 4
        bad = bad_ref[...]
        ot_tok = tok_rows(0, c)

        def inv_dft(b):
            z16 = pl.multiple_of((c * BPC + b) * 16, 16)
            zz = jnp.concatenate([zo[0:NR, lt, pl.ds(z16, 16), :].reshape(NF, 128) for lt in range(LT)], axis=1)
            return _mm(inv_ref[...], zz)

        ys = [inv_dft(0)]
        for b in range(BPC):
            rows = pl.ds(pl.multiple_of((c * BPC + b) * BLK, BLK), BLK)
            parts = []
            for j in range(NP):
                if b > 0 and j % 2 == 0:
                    ot[H + 1, ot_tok, 0:128] = ys[b - 1][j * 8:j * 8 + 8, _lanes(j * LT // NP)]
                ae = ot[2 * j, :, rows]
                ao = ot[2 * j + 1, :, rows]
                den = jnp.where(low, ao[0:8], ae[16:24])
                ok = (den >= DEN_LO) & (den <= DEN_HI)
                rec = 1.0 / den
                oe = ae * rec[4:5]
                oo = ao * rec[0:1]
                five = [oe[0:8], oe[8:16], jnp.where(low, oe[16:24], oo[0:8]), oo[8:16], oo[16:24]]
                for piece in five:
                    ok = ok & (jnp.abs(piece) <= OUT_HI)
                bad = jnp.where(ok, bad, 1.0)
                parts += five
            o = jnp.concatenate(parts, axis=0).T
            if b + 1 < BPC:
                ys.append(inv_dft(b + 1))
            att = _mm(o, wo_v[...])
            xf = x_v[rows, :].astype(F32)
            gate = jax.nn.sigmoid(jnp.sum(xf * gvec, axis=-1, keepdims=True))
            ssm = xf * (ys[b] + kv[rows, :] * dvec)
            out_v[rows, :] = (gate * att + (1.0 - gate) * ssm).astype(BF16)
            cp_o(c * BPC + b).start()
        bad_ref[...] = bad
        return carry

    def attempt(n, go):
        @pl.when(go > 0)
        def _():
            @pl.when(n > 0)
            def _():
                exact_attention()

            lax.fori_loop(0, NQ, final_body, 0)
            redo_ref[0] = (jnp.max(bad_ref[...]) > 0.0).astype(jnp.int32)
            for a in range(NB):
                cp_o(a).wait()

        return redo_ref[0]

    lax.fori_loop(0, 2, attempt, jnp.int32(1))


@jax.jit
def pallas_gated_mix__mha_block__ssm_conv_h3__prompt_kernel(
    A_x: jax.Array,
    A_wqkv: jax.Array,
    A_wo: jax.Array,
    B_q: jax.Array,
    B_k: jax.Array,
    B_v: jax.Array,
    B_shift_k: jax.Array,
    B_ssm_k: jax.Array,
    B_ssm_D: jax.Array,
    gate_w: jax.Array,
):
    del B_q
    fwd, inv = _dft_consts()
    hbm = pl.BlockSpec(memory_space=pl.ANY)
    scratch = [
        pltpu.VMEM((NIT, 32, TQ), U32),
        pltpu.VMEM((NIT, 32, TQ), F32),
        pltpu.VMEM((KR + QL * NV + 256, 128), U32),
        pltpu.VMEM((KR + QL * NV + 256, 128), U32),
        pltpu.VMEM((VTR + NV * DH + 256, 128), F32),
        pltpu.VMEM((VTR + NV * DH + 256, 128), F32),
        pltpu.VMEM((NP, NV, 128), F32),
        pltpu.VMEM((NR, LT, 2 * NB * 16, 128), F32),
        pltpu.VMEM((NR + 1, LT, NB * 16, 128), F32),
        pltpu.VMEM((CK // 2, TQ), U32),
        pltpu.VMEM((S, D), F32),
        pltpu.VMEM((NF, D), F32),
        pltpu.VMEM((S, D), BF16),
        pltpu.VMEM((S, D), BF16),
        pltpu.VMEM((NQ, D, TQ), BF16),
        pltpu.VMEM((S, D), BF16),
        pltpu.VMEM((H + 2, VR, S), F32),
        pltpu.VMEM((S + 32, D), BF16),
        pltpu.VMEM((3, D, D), BF16),
        pltpu.VMEM((D, D), BF16),
        pltpu.VMEM((D, D), BF16),
        pltpu.VMEM((8, TQ), U32),
        pltpu.VMEM((8, TQ), U32),
        pltpu.VMEM((8, TQ), F32),
        pltpu.VMEM((VR, TQ), F32),
        pltpu.VMEM((8, BLK), F32),
        pltpu.VMEM((NF, BLK), BF16),
        pltpu.VMEM((BLK, NF), BF16),
        pltpu.VMEM((KS, D), BF16),
        pltpu.VMEM((D,), BF16),
        pltpu.VMEM((D,), BF16),
        pltpu.SMEM((1,), jnp.int32),
        pltpu.SemaphoreType.DMA((7, NQ)),
        pltpu.SemaphoreType.DMA((NB,)),
    ]
    out = pl.pallas_call(
        _kernel,
        out_shape=jax.ShapeDtypeStruct((S, D), BF16),
        in_specs=[hbm] * 11,
        out_specs=hbm,
        scratch_shapes=scratch,
        compiler_params=pltpu.CompilerParams(vmem_limit_bytes=124 * 1024 * 1024),
        name="gated_mix_mha_h3",
    )(A_x.reshape(S, D), A_wqkv, A_wo, B_k.reshape(S, D), B_v.reshape(S, D), B_ssm_k,
      B_shift_k.T, B_ssm_D, gate_w, fwd, inv)
    return out.reshape(1, S, D)
```
